```python
import os as _os
_os.environ.setdefault("JAX_PLATFORMS", "cpu")
import jax
import jax.numpy as jnp

def _softmax(x, axis=-1):
    return jax.nn.softmax(x, axis=axis)
def _gelu(x):
    return jax.nn.gelu(x, approximate=True)
def _silu(x):
    return jax.nn.silu(x)
def _sigmoid(x):
    return jax.nn.sigmoid(x)
def _layernorm(x, axis=-1, eps=1e-5):
    m = jnp.mean(x, axis=axis, keepdims=True)
    v = jnp.var(x, axis=axis, keepdims=True)
    return (x - m) / jnp.sqrt(v + eps)
def _scatter_add(tgt, idx, src, axis=0):
    return tgt.at[idx].add(src)
def _segment_sum(src, seg, n):
    return jax.ops.segment_sum(src, seg, n)
class _Rng:
    def __init__(self, key):
        self._k = key
    def _next(self):
        self._k, sub = jax.random.split(self._k)
        return sub
    def normal(self, shape):
        return jax.random.normal(self._next(), shape, dtype=jnp.bfloat16)
    def randint(self, lo, hi, shape):
        return jax.random.randint(self._next(), shape, lo, hi, dtype=jnp.int32)
    def uniform(self, shape, lo=0.0, hi=1.0):
        return jax.random.uniform(self._next(), shape, jnp.bfloat16, lo, hi)
    def permutation(self, n):
        return jax.random.permutation(self._next(), n)


kernel_name = 'interleave_layers__gqa_block_cached__dense_activation_silu__decode'

def setup_inputs():
    _rng = _Rng(jax.random.key(int.from_bytes(__import__("os").urandom(4), "little")))
    _w = (lambda a: (lambda t: t.astype(jnp.bfloat16) if jnp.issubdtype(t.dtype, jnp.floating) else t)(jnp.asarray(a)))
    def _A_setup():
        B, Sq, D = 2, 1, 512
        Hq, Hkv, Sk, Dh = 32, 8, 8192, 128
        assert Hq % Hkv == 0, (Hq, Hkv)
        return {
            "x": _w((lambda *s: _rng.normal(s) * 0.1)(B, Sq, D)),
            "k_cache": _w((lambda *s: _rng.normal(s) * 0.8)(B, Hkv, Sk, Dh)),
            "v_cache": _w((lambda *s: _rng.normal(s) * 1.6)(B, Hkv, Sk, Dh)),
            "wq": _w((lambda *s: _rng.normal(s) * 0.8)(D, Hq * Dh) * (D ** -0.5)),
            "wo": _w((lambda *s: _rng.normal(s) * 1.6)(Hq * Dh, D) * ((Hq * Dh) ** -0.5)),
        }
    _A_in = _A_setup()

    def _B_setup():
        B, S, D, F = 2, 1, 512, 1792
        return {
            "x": _w((lambda *s: _rng.normal(s) * 0.1)(B, S, D)),
            "w1": _w((lambda *s: _rng.normal(s) * 0.4)(D, F) * (D ** -0.5)),
            "w2": _w((lambda *s: _rng.normal(s) * 0.4)(F, D) * (F ** -0.5)),
        }
    _B_in = _B_setup()

    return {
        "A_x": _A_in["x"],
        "A_k_cache": _A_in["k_cache"],
        "A_v_cache": _A_in["v_cache"],
        "A_wq": _A_in["wq"],
        "A_wo": _A_in["wo"],
        "B_x": _B_in["x"],
        "B_w1": _B_in["w1"],
        "B_w2": _B_in["w2"],
    }

def reference(A_x, A_k_cache, A_v_cache, A_wq, A_wo, B_x, B_w1, B_w2):
    def _A_ref(x, k_cache, v_cache, wq, wo):
        B, Sq, D = x.shape
        Hq, Dh = 32, 128
        Hkv = k_cache.shape[1]
        rep = Hq // Hkv
        q = (lambda x, *d: x.transpose(*d))((x @ wq).reshape(B, Sq, Hq, Dh), 0, 2, 1, 3)
        k = jnp.repeat(k_cache, rep, axis=1)
        v = jnp.repeat(v_cache, rep, axis=1)
        scores = jnp.einsum("bhqd,bhkd->bhqk", q, k) * (Dh ** -0.5)
        p = _softmax(scores, axis=-1)
        o = jnp.einsum("bhqk,bhkd->bhqd", p, v)
        return (lambda x, *d: x.transpose(*d))(o, 0, 2, 1, 3).reshape(B, Sq, Hq * Dh) @ wo

    def _B_ref(x, w1, w2):
        h = jnp.einsum("bsd,df->bsf", x, w1)
        h = _silu(h)
        out = jnp.einsum("bsf,fd->bsd", h, w2)
        return out

    x = A_x
    x = x + _A_ref(_layernorm(x, axis=-1), A_k_cache, A_v_cache, A_wq, A_wo)
    x = x + _B_ref(_layernorm(x, axis=-1), B_w1, B_w2)
    x = x + _A_ref(_layernorm(x, axis=-1), A_k_cache, A_v_cache, A_wq, A_wo)
    x = x + _B_ref(_layernorm(x, axis=-1), B_w1, B_w2)
    return x
```

```python
import functools
import jax
import jax.numpy as jnp
from jax import lax
import jax.experimental.pallas as pl
import jax.experimental.pallas.tpu as pltpu

B, D = 2, 512
HQ, HKV, SK, DH = 32, 8, 8192, 128
REP = HQ // HKV
F = 1792
EPS = 1e-5
SCALE = DH ** -0.5


def _ln(x):
    m = jnp.mean(x, axis=-1, keepdims=True)
    xc = x - m
    v = jnp.mean(xc * xc, axis=-1, keepdims=True)
    return xc * lax.rsqrt(v + EPS)


def _kernel(x_hbm, k_hbm, v_hbm, wq_hbm, wo_hbm, w1_hbm, w2_hbm, o_ref,
            xbuf, kbuf, vbuf, wq, wo, w1, w2, q_sc, oacc_sc, sem_w):
    cp_x = pltpu.make_async_copy(x_hbm, xbuf, sem_w.at[0])
    cp_wq = pltpu.make_async_copy(wq_hbm, wq, sem_w.at[1])
    cp_wo = pltpu.make_async_copy(wo_hbm, wo, sem_w.at[2])
    cp_w1 = pltpu.make_async_copy(w1_hbm, w1, sem_w.at[3])
    cp_w2 = pltpu.make_async_copy(w2_hbm, w2, sem_w.at[4])

    def cp_k(b, g):
        return pltpu.make_async_copy(k_hbm.at[b, g], kbuf.at[b, g], sem_w.at[5 + (b * HKV + g) * 2])

    def cp_v(b, g):
        return pltpu.make_async_copy(v_hbm.at[b, g], vbuf.at[b, g], sem_w.at[6 + (b * HKV + g) * 2])

    cp_x.start()
    cp_wq.start()
    for g in range(HKV):
        cp_k(0, g).start()
        cp_v(0, g).start()
    cp_wo.start()
    cp_w1.start()
    cp_w2.start()
    for g in range(HKV):
        cp_k(1, g).start()
        cp_v(1, g).start()

    row = lax.broadcasted_iota(jnp.int32, (8, DH), 0)

    def compute_q(x):
        h = _ln(x).astype(jnp.bfloat16)
        q = jnp.dot(h, wq[...], preferred_element_type=jnp.float32) * SCALE
        for g in range(HKV):
            qg = jnp.zeros((8, DH), jnp.float32)
            for r in range(REP):
                c = (g * REP + r) * DH
                qg = jnp.where(row == r, q[:, c:c + DH], qg)
            q_sc[g] = qg.astype(jnp.bfloat16)

    def attention(b, wait):
        def body(g, carry):
            if wait:
                cp_k(b, g).wait()
            qg = q_sc[g]
            s = lax.dot_general(qg, kbuf[b, g], (((1,), (1,)), ((), ())),
                                preferred_element_type=jnp.float32)
            m = jnp.max(s, axis=1, keepdims=True)
            p = jnp.exp(s - m)
            l = jnp.sum(p, axis=1, keepdims=True)
            if wait:
                cp_v(b, g).wait()
            o = jnp.dot(p.astype(jnp.bfloat16), vbuf[b, g], preferred_element_type=jnp.float32)
            o = o / l
            for r in range(REP):
                oacc_sc[g * REP + r] = jnp.where(row == r, o, 0.0).astype(jnp.bfloat16)
            return carry
        lax.fori_loop(0, HKV, body, 0)

    def out_proj():
        ofull = jnp.concatenate([oacc_sc[i] for i in range(HQ)], axis=1)
        y = jnp.dot(ofull, wo[...], preferred_element_type=jnp.float32)
        y = jnp.sum(y, axis=0, keepdims=True)
        return jnp.broadcast_to(y, (8, D))

    def ffn(x):
        h = _ln(x).astype(jnp.bfloat16)
        a = jnp.dot(h, w1[...], preferred_element_type=jnp.float32)
        a = a * jax.nn.sigmoid(a)
        return jnp.dot(a.astype(jnp.bfloat16), w2[...], preferred_element_type=jnp.float32)

    cp_x.wait()
    cp_wq.wait()
    xs = xbuf[...].astype(jnp.float32)
    for b in range(B):
        x = jnp.broadcast_to(xs[b:b + 1, :], (8, D))
        with jax.named_scope(f"q1_{b}"):
            compute_q(x)
        with jax.named_scope(f"att1_{b}"):
            attention(b, True)
        with jax.named_scope(f"wo1_{b}"):
            if b == 0:
                cp_wo.wait()
            x = x + out_proj()
        with jax.named_scope(f"ffn1_{b}"):
            if b == 0:
                cp_w1.wait()
                cp_w2.wait()
            x = x + ffn(x)
        with jax.named_scope(f"q2_{b}"):
            compute_q(x)
        with jax.named_scope(f"att2_{b}"):
            attention(b, False)
        with jax.named_scope(f"wo2_{b}"):
            x = x + out_proj()
        with jax.named_scope(f"ffn2_{b}"):
            x = x + ffn(x)
        o_ref[b:b + 1, :] = x[0:1, :].astype(o_ref.dtype)


@jax.jit
def pallas_interleave_layers__gqa_block_cached__dense_activation_silu__decode_kernel(A_x, A_k_cache, A_v_cache, A_wq, A_wo, B_x, B_w1, B_w2):
    x2 = A_x.reshape(B, D)
    any_spec = pl.BlockSpec(memory_space=pl.ANY)
    out = pl.pallas_call(
        _kernel,
        out_shape=jax.ShapeDtypeStruct((B, D), jnp.bfloat16),
        in_specs=[any_spec] * 7,
        out_specs=pl.BlockSpec(memory_space=pltpu.VMEM),
        scratch_shapes=[
            pltpu.VMEM((B, D), jnp.bfloat16),
            pltpu.VMEM((B, HKV, SK, DH), jnp.bfloat16),
            pltpu.VMEM((B, HKV, SK, DH), jnp.bfloat16),
            pltpu.VMEM((D, HQ * DH), jnp.bfloat16),
            pltpu.VMEM((HQ * DH, D), jnp.bfloat16),
            pltpu.VMEM((D, F), jnp.bfloat16),
            pltpu.VMEM((F, D), jnp.bfloat16),
            pltpu.VMEM((HKV, 8, DH), jnp.bfloat16),
            pltpu.VMEM((HQ, 8, DH), jnp.bfloat16),
            pltpu.SemaphoreType.DMA((5 + 2 * B * HKV,)),
        ],
        compiler_params=pltpu.CompilerParams(vmem_limit_bytes=110 * 1024 * 1024),
    )(x2, A_k_cache, A_v_cache, A_wq, A_wo, B_w1, B_w2)
    return out.reshape(B, 1, D)
```

```python
import jax
import jax.numpy as jnp
from jax import lax
import jax.experimental.pallas as pl
import jax.experimental.pallas.tpu as pltpu

B, D = 2, 512
HQ, HKV, SK, DH = 32, 8, 8192, 128
REP = HQ // HKV
GW = REP * DH
F = 1792
EPS = 1e-5
SCALE = DH ** -0.5
LOG2E = 1.4426950408889634
NT = SK // 128
ND = D // 128
NJ = F // 128
bf16 = jnp.bfloat16
f32 = jnp.float32
u32 = jnp.uint32

ROWS = (3, 7, 1, 5)
LASTP = (32, 16, 8, 4, 4)
TB = 32
QMXU = 1
HV = 6
PJ = 6
LAG = 28
SMG = 8
Q1A, Q1B = 36, 58
SMA, SMB = 36, 4


def _stats(x):
    m = jnp.mean(x, axis=-1, keepdims=True)
    xc = x - m
    v = jnp.mean(xc * xc, axis=-1, keepdims=True)
    return m, lax.rsqrt(v + EPS)


def _stats1(x, c):
    d = x - c
    s1 = jnp.mean(d, axis=-1, keepdims=True)
    s2 = jnp.mean(d * d, axis=-1, keepdims=True)
    v = jnp.maximum(s2 - s1 * s1, 0.0)
    return c + s1, lax.rsqrt(v + EPS)


def _silu_half(h):
    return h + h * jnp.tanh(h)


def _rnd(x):
    xb = x.astype(bf16)
    return xb, xb.astype(f32)


def _acc(a, t):
    return t if a is None else a + t


def _kernel(x_hbm, k_hbm, v_hbm, wq_hbm, wo_hbm, w1_hbm, w2_hbm, o_ref,
            xbuf, k0buf, k1buf, vbuf, wq, wo, w1, w2,
            wqt, wot, w1t, w2t, wqf, wof, w1f, w2f, cq, c1,
            q_sc, p_sc, l_sc, y_sc, o_sc, hb_sc, z_sc, *ob_sc):
    z_sc[0] = 0
    row = lax.broadcasted_iota(jnp.int32, (8, DH), 0)
    k_u = k0buf.bitcast(u32)
    v_u = vbuf.bitcast(u32)

    def as_bf(x):
        return pltpu.bitcast(x, bf16)

    def mm(a, w_u32):
        return jnp.dot(a, as_bf(w_u32), preferred_element_type=f32)

    def pick_rows(parts):
        qg = parts[0]
        for r in range(1, REP):
            qg = jnp.where(row == ROWS[r], parts[r], qg)
        return qg

    def fold4(acc):
        a = [x + pltpu.roll(x, 4, 0) for x in acc]
        b01 = jnp.where(row < 4, a[0], a[1])
        b23 = jnp.where(row < 4, a[2], a[3])
        c01 = b01 + pltpu.roll(b01, 2, 0)
        c23 = b23 + pltpu.roll(b23, 6, 0)
        d = jnp.where((row & 2) == 2, c01, c23)
        return d + pltpu.roll(d, 1, 0)

    def q_raw_mxu(xb, m, g):
        return pick_rows([mm(xb, wqt[g * REP + r]) for r in range(REP)]) - m * cq[g]

    def softmax(s):
        m = jnp.max(s, axis=1, keepdims=True)
        p = jnp.exp(s - m)
        l = jnp.sum(p, axis=1, keepdims=True)
        return p.astype(bf16), l

    def o_expand(o):
        return jnp.concatenate([jnp.where(row == ROWS[r], o, 0.0).astype(bf16) for r in range(REP)], axis=1)

    def rowsum(y):
        return jnp.broadcast_to(jnp.sum(y, axis=0, keepdims=True), (8, D))

    def wo_mxu(oe, g):
        return jnp.concatenate([mm(oe, wot[n, pl.ds(g * (GW // 2), GW // 2), :]) for n in range(ND)], axis=1)

    def ffn(x):
        xb, xf = _rnd(x)
        m, rs = _stats(xf)
        a = jnp.concatenate([mm(xb, w1t[j]) for j in range(NJ)], axis=1)
        a = (a - m * c1[...]) * rs
        a = (a * jax.nn.sigmoid(a)).astype(bf16)
        return xf + jnp.concatenate([mm(a, w2t[n]) for n in range(ND)], axis=1)

    def colb(v):
        return jnp.broadcast_to(v, (128, 128)).T

    def after(v, dep, zmask):
        return pltpu.bitcast(pltpu.bitcast(v, u32) | (pltpu.bitcast(dep, u32) & zmask), f32)

    def ffn_fast(x, c, zmask):
        xb, xf = _rnd(x)
        m, rs = _stats1(xf, c)
        rs = rs * 0.5
        NM = NJ - HV
        x0p = after(xf[:, 0:128], jnp.broadcast_to(rs, (8, 128)), zmask)
        xbp = jnp.concatenate([x0p.astype(bf16), xb[:, 128:]], axis=1)
        pre = [mm(xb if j < PJ else xbp, w1t[j]) for j in range(NM)]
        yv = [None] * ND
        for rb in range(HV * 16):
            acc = None
            for c_ in range(ND):
                acc = _acc(acc, w1f[rb * 8:(rb + 1) * 8, c_ * 128:(c_ + 1) * 128] * xf[:, c_ * 128:(c_ + 1) * 128])
            a = jnp.broadcast_to(jnp.sum(acc, axis=1, keepdims=True), (8, 128))
            a = _silu_half(a * rs)
            for n in range(ND):
                yv[n] = _acc(yv[n], w2f[rb * 8:(rb + 1) * 8, n * 128:(n + 1) * 128] * a)
        y = [None] * ND
        for j in range(NM):
            a = (pre[j] - m * c1[:, j * 128:(j + 1) * 128]) * rs
            a = _silu_half(a).astype(bf16)
            for n in range(ND):
                y[n] = _acc(y[n], mm(a, w2t[n, j * 64:(j + 1) * 64, :]))
        xf = xf + rowsum(jnp.concatenate(yv, axis=1))
        return xf + jnp.concatenate(y, axis=1), m

    NSEM = 5 + 2 * B * HKV + len(LASTP)

    def streamed(sem):
        cp_x = pltpu.make_async_copy(x_hbm, xbuf, sem.at[0])
        cp_wq = pltpu.make_async_copy(wq_hbm, wq, sem.at[1])
        cp_wo = pltpu.make_async_copy(wo_hbm, wo, sem.at[2])
        cp_w1 = pltpu.make_async_copy(w1_hbm, w1, sem.at[3])
        cp_w2 = pltpu.make_async_copy(w2_hbm, w2, sem.at[4])

        def cp_k(b, g):
            return pltpu.make_async_copy(k_hbm.at[b, g], (k0buf, k1buf)[b].at[g], sem.at[5 + (b * HKV + g) * 2])

        def cp_v(b, g):
            return pltpu.make_async_copy(v_hbm.at[b, g], vbuf.at[b, g], sem.at[6 + (b * HKV + g) * 2])

        def cp_vlast(c):
            r0 = sum(LASTP[:c]) * 128
            n = LASTP[c] * 128
            return pltpu.make_async_copy(v_hbm.at[1, HKV - 1, pl.ds(r0, n)],
                                         vbuf.at[1, HKV - 1, pl.ds(r0, n)],
                                         sem.at[5 + 2 * B * HKV + c])

        cp_x.start()
        cp_wq.start()
        for g in range(HKV):
            cp_k(0, g).start()
            cp_v(0, g).start()
        cp_wo.start()
        cp_w1.start()
        cp_w2.start()
        for g in range(HKV):
            cp_k(1, g).start()
        for g in range(HKV - 1):
            cp_v(1, g).start()
        for c in range(len(LASTP)):
            cp_vlast(c).start()

        ones = jnp.ones((8, D), bf16)

        def compute_q(x, slot):
            xb, xf = _rnd(x)
            m, rs = _stats(xf)
            for g in range(HKV):
                q_sc[slot, g] = (q_raw_mxu(xb, m, g) * (rs * SCALE)).astype(bf16)

        def attention0(wait):
            def body(g, carry):
                if wait:
                    cp_k(0, g).wait()
                s = lax.dot_general(q_sc[0, g], k0buf[g], (((1,), (1,)), ((), ())),
                                    preferred_element_type=f32)
                p, l = softmax(s)
                if wait:
                    cp_v(0, g).wait()
                o = jnp.dot(p, vbuf[0, g], preferred_element_type=f32) / l
                p_sc[g, :, 0:GW] = o_expand(o)
                return carry
            lax.fori_loop(0, HKV, body, 0)

        def out_proj0():
            ofull = jnp.concatenate([p_sc[g, :, 0:GW] for g in range(HKV)], axis=1)
            return rowsum(jnp.dot(ofull, wo[...], preferred_element_type=f32))

        cp_x.wait()
        cp_wq.wait()
        xs = xbuf[...].astype(f32)
        x0 = jnp.broadcast_to(xs[0:1, :], (8, D))
        x1 = jnp.broadcast_to(xs[1:2, :], (8, D))

        def prep_q(j, carry):
            w = wq[:, pl.ds(pl.multiple_of(j * 128, 128), 128)]
            wqt[j] = pltpu.bitcast(w, u32)
            wqf[j] = w.astype(f32)
            return carry
        lax.fori_loop(0, HQ, prep_q, 0)
        for g in range(HKV):
            cq[g] = pick_rows([mm(ones, wqt[g * REP + r]) for r in range(REP)])
        compute_q(x0, 0)
        compute_q(x1, 1)
        attention0(True)
        cp_wo.wait()
        x0 = x0 + out_proj0()

        def prep_o(i, carry):
            w = wo[pl.ds(pl.multiple_of(i * 128, 128), 128), :]
            wof[i] = w.astype(f32)
            for n in range(ND):
                wot[n, pl.ds(pl.multiple_of(i * 64, 64), 64), :] = pltpu.bitcast(w[:, n * 128:(n + 1) * 128], u32)
            return carry
        lax.fori_loop(0, HQ, prep_o, 0)
        cp_w1.wait()
        cp_w2.wait()
        for j in range(NJ):
            w1t[j] = pltpu.bitcast(w1[:, j * 128:(j + 1) * 128], u32)
        for n in range(ND):
            w2t[n] = pltpu.bitcast(w2[:, n * 128:(n + 1) * 128], u32)
        c1[...] = jnp.dot(ones, w1[...], preferred_element_type=f32)
        for r in range(HV):
            j = NJ - HV + r
            w1f[r * 128:(r + 1) * 128, :] = (w1[:, j * 128:(j + 1) * 128].astype(f32)
                                             - c1[0:1, j * 128:(j + 1) * 128] * (1.0 / D)).T
            w2f[r * 128:(r + 1) * 128, :] = w2[j * 128:(j + 1) * 128, :].astype(f32)
        x0 = ffn(x0)
        compute_q(x0, 0)
        attention0(False)
        x0 = _rnd(x0)[1] + out_proj0()
        x0 = ffn(x0)
        o_ref[0:1, :] = x0[0:1, :].astype(o_ref.dtype)

        def kbody(g, carry):
            cp_k(1, g).wait()

            def tbody(c, carry2):
                for t in range(TB):
                    r0 = pl.multiple_of((c * TB + t) * 128, 128)
                    k0buf[g, pl.ds(r0, 128), :] = k1buf[g, pl.ds(r0, 128), :].T
                return carry2
            lax.fori_loop(0, NT // TB, tbody, 0)
            qg = q_sc[1, g]
            s = jnp.concatenate([mm(qg, k_u[g, t * 64:(t + 1) * 64, :]) for t in range(NT)], axis=1)
            p, l = softmax(s)
            p_sc[g] = p
            l_sc[g] = jnp.broadcast_to(1.0 / l, (8, DH))
            return carry
        lax.fori_loop(0, HKV, kbody, 0)

        y_sc[...] = jnp.zeros((8, D), f32)

        def vbody(g, carry):
            cp_v(1, g).wait()
            o = mm(p_sc[g], v_u[1, g]) * l_sc[g]
            y_sc[...] += wo_mxu(o_expand(o), g)
            return carry
        lax.fori_loop(0, HKV - 1, vbody, 0)
        g = HKV - 1
        o = jnp.zeros((8, DH), f32)
        for c in range(len(LASTP)):
            t0 = sum(LASTP[:c])
            t1 = t0 + LASTP[c]
            cp_vlast(c).wait()
            o = o + mm(p_sc[g, :, t0 * 128:t1 * 128], v_u[1, g, t0 * 64:t1 * 64, :])
        o_sc[...] = o

    pl.run_scoped(streamed, pltpu.SemaphoreType.DMA((NSEM,)))

    z8 = pl.multiple_of(z_sc[0] * 8, 8)
    zmask = jnp.full((8, 128), z_sc[0], jnp.int32).astype(u32)
    g = HKV - 1
    x1 = jnp.broadcast_to(xbuf[...].astype(f32)[1:2, :], (8, D))
    o = o_sc[...] * l_sc[g]
    y = y_sc[...] + wo_mxu(o_expand(o), g)
    m = jnp.mean(x1, axis=-1, keepdims=True)
    x1 = x1 + rowsum(y)
    x1, m = ffn_fast(x1, m, zmask)
    xb, xf = _rnd(x1)
    m, rs = _stats1(xf, m)
    csc = rs * (SCALE * LOG2E)
    qs = [None] * HKV
    res = []
    clock = [0]

    def tied(v):
        i = clock[0] - LAG
        return v if i < 0 else after(v, res[i], zmask)

    for g in range(QMXU):
        qs[g] = _rnd(q_raw_mxu(xb, m, g))[1]
    for c in range(ND):
        hb_sc[c * 128:(c + 1) * 128, :] = colb(xf[0:1, c * 128:(c + 1) * 128])

    def q_task(g):
        acc = [None] * REP
        for kb in range(D // 8):
            hv = tied(hb_sc[pl.ds(z8 + kb * 8, 8), :])
            for r in range(REP):
                acc[r] = _acc(acc[r], wqf[g * REP + r, kb * 8:(kb + 1) * 8, :] * hv)
            yield acc[kb % REP]
        qs[g] = _rnd(fold4(acc) - m * cq[g])[1]

    yacc = [None] * ND

    def o_task(g):
        for r in range(REP):
            for kb in range(DH // 8):
                ov = tied(ob_sc[g][r, pl.ds(z8 + kb * 8, 8), :])
                for n in range(ND):
                    yacc[n] = _acc(yacc[n], wof[g * REP + r, kb * 8:(kb + 1) * 8, n * 128:(n + 1) * 128] * ov)
                yield yacc[kb % ND]

    ss = [[None] * NT for _ in range(HKV)]
    ps = [None] * HKV
    ls = [None] * HKV

    def sm_task(g):
        s = ss[g]
        mx = s[0]
        for t in range(1, NT):
            mx = jnp.maximum(mx, s[t])
        mx = jnp.broadcast_to(jnp.max(mx, axis=1, keepdims=True), (8, 128))
        out = []
        lacc = None
        for t0 in range(0, NT, SMG):
            mxt = tied(mx)
            es = [jnp.exp2((s[t] - mxt) * csc) for t in range(t0, t0 + SMG)]
            out += es
            while len(es) > 1:
                es = [es[i] + es[i + 1] for i in range(0, len(es), 2)]
            lacc = _acc(lacc, es[0])
            yield lacc
        ps[g] = out
        ls[g] = jnp.sum(lacc, axis=1, keepdims=True)

    stages = [("qk", 0)]
    for g in range(HKV):
        if g + 1 < HKV:
            stages.append(("qk", g + 1))
        stages.append(("pv", g))
    start = {st: i * NT for i, st in enumerate(stages)}
    end = {st: (i + 1) * NT for i, st in enumerate(stages)}

    tasks = []
    for g in range(QMXU, HKV):
        t0, t1 = (Q1A, Q1B) if g == 1 else (start[("qk", g - 1)], end[("qk", g - 1)])
        tasks.append([q_task(g), D // 8, t0, t1, 0])
    for g in range(HKV - 2):
        tasks.append([o_task(g), REP * DH // 8, start[("pv", g + 1)], end[("pv", g + 1)], 0])
    for g in range(HKV):
        st = ("qk", g + 1) if g + 1 < HKV else ("pv", g - 1)
        tasks.append([sm_task(g), NT // SMG, end[st] - SMA, end[st] - SMB, 0])

    def pinned(lhs):
        tau = clock[0]
        bits = None
        for tk in tasks:
            gen, n, t0, t1, done = tk
            if tau < t0 or done > n:
                continue
            want = n + 1 if tau >= t1 else (n * (tau - t0 + 1)) // (t1 - t0)
            pin = None
            while tk[4] < want:
                pin = next(gen, None)
                tk[4] += 1
            if pin is not None:
                pb = pltpu.bitcast(pin, u32)
                bits = pb if bits is None else bits | pb
        if bits is not None:
            lhs = pltpu.bitcast(pltpu.bitcast(lhs, u32) | (bits & zmask), f32)
        clock[0] += 1
        return lhs.astype(bf16)

    for kind, g in stages:
        if kind == "qk":
            for t in range(NT):
                ss[g][t] = mm(pinned(qs[g]), k_u[g, t * 64:(t + 1) * 64, :])
                res.append(ss[g][t])
        else:
            acc = [None] * 4
            for t in range(NT):
                d = mm(pinned(ps[g][t]), v_u[1, g, t * 64:(t + 1) * 64, :])
                res.append(d)
                acc[t % 4] = _acc(acc[t % 4], d)
            o = ((acc[0] + acc[1]) + (acc[2] + acc[3])) / ls[g]
            if g < HKV - 1:
                ob16 = _rnd(o)[1]
                for r in range(REP):
                    ob_sc[g][r] = colb(ob16[ROWS[r]:ROWS[r] + 1, :])
    for tk in tasks:
        for _ in tk[0]:
            pass
    for _ in o_task(HKV - 2):
        pass
    y = jnp.concatenate(yacc, axis=1) + wo_mxu(o_expand(o), HKV - 1)
    x1 = xf + rowsum(y)
    x1, _ = ffn_fast(x1, m, zmask)
    o_ref[1:2, :] = x1[0:1, :].astype(o_ref.dtype)


@jax.jit
def pallas_interleave_layers__gqa_block_cached__dense_activation_silu__decode_kernel(A_x, A_k_cache, A_v_cache, A_wq, A_wo, B_x, B_w1, B_w2):
    x2 = A_x.reshape(B, D)
    any_spec = pl.BlockSpec(memory_space=pl.ANY)
    out = pl.pallas_call(
        _kernel,
        out_shape=jax.ShapeDtypeStruct((B, D), bf16),
        in_specs=[any_spec] * 7,
        out_specs=pl.BlockSpec(memory_space=pltpu.VMEM),
        scratch_shapes=[
            pltpu.VMEM((B, D), bf16),
            pltpu.VMEM((HKV, SK, DH), bf16),
            pltpu.VMEM((HKV, SK, DH), bf16),
            pltpu.VMEM((B, HKV, SK, DH), bf16),
            pltpu.VMEM((D, HQ * DH), bf16),
            pltpu.VMEM((HQ * DH, D), bf16),
            pltpu.VMEM((D, F), bf16),
            pltpu.VMEM((F, D), bf16),
            pltpu.VMEM((HQ, D // 2, 128), u32),
            pltpu.VMEM((ND, HQ * DH // 2, 128), u32),
            pltpu.VMEM((NJ, D // 2, 128), u32),
            pltpu.VMEM((ND, F // 2, 128), u32),
            pltpu.VMEM((HQ, D, 128), f32),
            pltpu.VMEM((HQ, DH, D), f32),
            pltpu.VMEM((HV * 128, D), f32),
            pltpu.VMEM((HV * 128, D), f32),
            pltpu.VMEM((HKV, 8, DH), f32),
            pltpu.VMEM((8, F), f32),
            pltpu.VMEM((B, HKV, 8, DH), bf16),
            pltpu.VMEM((HKV, 8, SK), bf16),
            pltpu.VMEM((HKV, 8, DH), f32),
            pltpu.VMEM((8, D), f32),
            pltpu.VMEM((8, DH), f32),
            pltpu.VMEM((D, 128), f32),
            pltpu.SMEM((1,), jnp.int32),
        ] + [pltpu.VMEM((REP, DH, 128), f32)] * (HKV - 1),
        compiler_params=pltpu.CompilerParams(vmem_limit_bytes=124 * 1024 * 1024),
    )(x2, A_k_cache, A_v_cache, A_wq, A_wo, B_w1, B_w2)
    return out.reshape(B, 1, D)
```

```python
import jax
import jax.numpy as jnp
from jax import lax
import jax.experimental.pallas as pl
import jax.experimental.pallas.tpu as pltpu

B, D = 2, 512
HQ, HKV, SK, DH = 32, 8, 8192, 128
REP = HQ // HKV
GW = REP * DH
F = 1792
EPS = 1e-5
SCALE = DH ** -0.5
LOG2E = 1.4426950408889634
NT = SK // 128
ND = D // 128
NJ = F // 128
bf16 = jnp.bfloat16
f32 = jnp.float32
u32 = jnp.uint32

ROWS = (3, 7, 1, 5)
LASTP = (32, 16, 8, 4, 4)
TB = 32
QMXU = 1
HV = 6
PJ = 6
LAG = 26
SMG = 8
Q1A, Q1B = 36, 58
SMA, SMB = 32, 2
XA, XB = 4, 4
XV = (0, 0, XA, XA, XA, XA, XA, XB)
XT = 2
XVMAX = max(max(XV), 1)
TG, PG = 4, 2
CBA, CBB = 0, 24
O6A, O6B, O6L = 4, 28, 12


def _stats(x):
    m = jnp.mean(x, axis=-1, keepdims=True)
    xc = x - m
    v = jnp.mean(xc * xc, axis=-1, keepdims=True)
    return m, lax.rsqrt(v + EPS)


def _stats1(x, c):
    d = x - c
    s1 = jnp.mean(d, axis=-1, keepdims=True)
    s2 = jnp.mean(d * d, axis=-1, keepdims=True)
    v = jnp.maximum(s2 - s1 * s1, 0.0)
    return c + s1, lax.rsqrt(v + EPS)


def _silu_half(h):
    return h + h * jnp.tanh(h)


def _rnd(x):
    xb = x.astype(bf16)
    return xb, xb.astype(f32)


def _acc(a, t):
    return t if a is None else a + t


def _kernel(x_hbm, k_hbm, v_hbm, wq_hbm, wo_hbm, w1_hbm, w2_hbm, o_ref,
            xbuf, k0buf, k1buf, vbuf, wq, wo, w1, w2,
            wqt, wot, w1t, w2t, wqf, wof, w1f, w2f, cq, c1,
            q_sc, p_sc, l_sc, y_sc, o_sc, hb_sc, z_sc, ktf, *bsc):
    ob_sc = bsc[:HKV - 1]
    qb_sc = bsc[HKV - 1:]
    z_sc[0] = 0
    row = lax.broadcasted_iota(jnp.int32, (8, DH), 0)

    def as_bf(x):
        return pltpu.bitcast(x, bf16)

    def mm(a, w_u32):
        return jnp.dot(a, as_bf(w_u32), preferred_element_type=f32)

    def pick_rows(parts):
        qg = parts[0]
        for r in range(1, REP):
            qg = jnp.where(row == ROWS[r], parts[r], qg)
        return qg

    def fold4(acc):
        a = [x + pltpu.roll(x, 4, 0) for x in acc]
        b01 = jnp.where(row < 4, a[0], a[1])
        b23 = jnp.where(row < 4, a[2], a[3])
        c01 = b01 + pltpu.roll(b01, 2, 0)
        c23 = b23 + pltpu.roll(b23, 6, 0)
        d = jnp.where((row & 2) == 2, c01, c23)
        return d + pltpu.roll(d, 1, 0)

    def q_raw_mxu(xb, m, g):
        return pick_rows([mm(xb, wqt[g * REP + r]) for r in range(REP)]) - m * cq[g]

    def softmax(s):
        m = jnp.max(s, axis=1, keepdims=True)
        p = jnp.exp(s - m)
        l = jnp.sum(p, axis=1, keepdims=True)
        return p.astype(bf16), l

    def o_expand(o):
        return jnp.concatenate([jnp.where(row == ROWS[r], o, 0.0).astype(bf16) for r in range(REP)], axis=1)

    def rowsum(y):
        return jnp.broadcast_to(jnp.sum(y, axis=0, keepdims=True), (8, D))

    def wo_mxu(oe, g):
        return jnp.concatenate([mm(oe, wot[n, pl.ds(g * (GW // 2), GW // 2), :]) for n in range(ND)], axis=1)

    def ffn(x):
        xb, xf = _rnd(x)
        m, rs = _stats(xf)
        a = jnp.concatenate([mm(xb, w1t[j]) for j in range(NJ)], axis=1)
        a = (a - m * c1[...]) * rs
        a = (a * jax.nn.sigmoid(a)).astype(bf16)
        return xf + jnp.concatenate([mm(a, w2t[n]) for n in range(ND)], axis=1)

    def colb(v):
        return jnp.broadcast_to(v, (128, 128)).T

    def after(v, dep, zmask):
        return pltpu.bitcast(pltpu.bitcast(v, u32) | (pltpu.bitcast(dep, u32) & zmask), f32)

    def ffn_fast(x, c, zmask):
        xb, xf = _rnd(x)
        m, rs = _stats1(xf, c)
        rs = rs * 0.5
        NM = NJ - HV
        x0p = after(xf[:, 0:128], jnp.broadcast_to(rs, (8, 128)), zmask)
        xbp = jnp.concatenate([x0p.astype(bf16), xb[:, 128:]], axis=1)
        pre = [mm(xb if j < PJ else xbp, w1t[j]) for j in range(NM)]
        yv = [None] * ND
        for rb in range(HV * 16):
            acc = None
            for c_ in range(ND):
                acc = _acc(acc, w1f[rb * 8:(rb + 1) * 8, c_ * 128:(c_ + 1) * 128] * xf[:, c_ * 128:(c_ + 1) * 128])
            a = jnp.broadcast_to(jnp.sum(acc, axis=1, keepdims=True), (8, 128))
            a = _silu_half(a * rs)
            for n in range(ND):
                yv[n] = _acc(yv[n], w2f[rb * 8:(rb + 1) * 8, n * 128:(n + 1) * 128] * a)
        y = [None] * ND
        for j in range(NM):
            a = (pre[j] - m * c1[:, j * 128:(j + 1) * 128]) * rs
            a = _silu_half(a).astype(bf16)
            for n in range(ND):
                y[n] = _acc(y[n], mm(a, w2t[n, j * 64:(j + 1) * 64, :]))
        xf = xf + rowsum(jnp.concatenate(yv, axis=1))
        return xf + jnp.concatenate(y, axis=1), m

    NSEM = 5 + 2 * B * HKV + len(LASTP)

    def streamed(sem):
        cp_x = pltpu.make_async_copy(x_hbm, xbuf, sem.at[0])
        cp_wq = pltpu.make_async_copy(wq_hbm, wq, sem.at[1])
        cp_wo = pltpu.make_async_copy(wo_hbm, wo, sem.at[2])
        cp_w1 = pltpu.make_async_copy(w1_hbm, w1, sem.at[3])
        cp_w2 = pltpu.make_async_copy(w2_hbm, w2, sem.at[4])

        def cp_k(b, g):
            return pltpu.make_async_copy(k_hbm.at[b, g], (k0buf, k1buf)[b].at[g], sem.at[5 + (b * HKV + g) * 2])

        def cp_v(b, g):
            return pltpu.make_async_copy(v_hbm.at[b, g], vbuf.at[b, g], sem.at[6 + (b * HKV + g) * 2])

        def cp_vlast(c):
            r0 = sum(LASTP[:c]) * 128
            n = LASTP[c] * 128
            return pltpu.make_async_copy(v_hbm.at[1, HKV - 1, pl.ds(r0, n)],
                                         vbuf.at[1, HKV - 1, pl.ds(r0, n)],
                                         sem.at[5 + 2 * B * HKV + c])

        cp_wq.start()
        cp_x.start()
        for g in range(HKV):
            cp_k(0, g).start()
            cp_v(0, g).start()
        cp_wo.start()
        cp_w1.start()
        cp_w2.start()
        for g in range(HKV):
            cp_k(1, g).start()
        for g in range(HKV - 1):
            cp_v(1, g).start()
        for c in range(len(LASTP)):
            cp_vlast(c).start()

        ones = jnp.ones((8, D), bf16)

        def compute_q(x, slot):
            xb, xf = _rnd(x)
            m, rs = _stats(xf)
            for g in range(HKV):
                q_sc[slot, g] = (q_raw_mxu(xb, m, g) * (rs * SCALE)).astype(bf16)

        def attention0(wait):
            def body(g, carry):
                if wait:
                    cp_k(0, g).wait()
                s = lax.dot_general(q_sc[0, g], k0buf[g], (((1,), (1,)), ((), ())),
                                    preferred_element_type=f32)
                p, l = softmax(s)
                if wait:
                    cp_v(0, g).wait()
                o = jnp.dot(p, vbuf[0, g], preferred_element_type=f32) / l
                p_sc[g, :, 0:GW] = o_expand(o)
                return carry
            lax.fori_loop(0, HKV, body, 0)

        def out_proj0():
            ofull = jnp.concatenate([p_sc[g, :, 0:GW] for g in range(HKV)], axis=1)
            return rowsum(jnp.dot(ofull, wo[...], preferred_element_type=f32))

        cp_x.wait()
        cp_wq.wait()
        xs = xbuf[...].astype(f32)
        x0 = jnp.broadcast_to(xs[0:1, :], (8, D))
        x1 = jnp.broadcast_to(xs[1:2, :], (8, D))

        def prep_q(j, carry):
            w = wq[:, pl.ds(pl.multiple_of(j * 128, 128), 128)]
            wqt[j] = pltpu.bitcast(w, u32)
            wqf[j] = w.astype(f32)
            return carry
        lax.fori_loop(0, HQ, prep_q, 0)
        for g in range(HKV):
            cq[g] = pick_rows([mm(ones, wqt[g * REP + r]) for r in range(REP)])
        compute_q(x0, 0)
        compute_q(x1, 1)
        attention0(True)
        cp_wo.wait()
        x0 = x0 + out_proj0()

        def prep_o(i, carry):
            w = wo[pl.ds(pl.multiple_of(i * 128, 128), 128), :]
            wof[i] = w.astype(f32)
            for n in range(ND):
                wot[n, pl.ds(pl.multiple_of(i * 64, 64), 64), :] = pltpu.bitcast(w[:, n * 128:(n + 1) * 128], u32)
            return carry
        lax.fori_loop(0, HQ, prep_o, 0)
        cp_w1.wait()
        cp_w2.wait()
        for j in range(NJ):
            w1t[j] = pltpu.bitcast(w1[:, j * 128:(j + 1) * 128], u32)
        for n in range(ND):
            w2t[n] = pltpu.bitcast(w2[:, n * 128:(n + 1) * 128], u32)
        c1[...] = jnp.dot(ones, w1[...], preferred_element_type=f32)
        for r in range(HV):
            j = NJ - HV + r
            w1f[r * 128:(r + 1) * 128, :] = (w1[:, j * 128:(j + 1) * 128].astype(f32)
                                             - c1[0:1, j * 128:(j + 1) * 128] * (1.0 / D)).T
            w2f[r * 128:(r + 1) * 128, :] = w2[j * 128:(j + 1) * 128, :].astype(f32)
        x0 = ffn(x0)
        compute_q(x0, 0)
        attention0(False)
        x0 = _rnd(x0)[1] + out_proj0()
        x0 = ffn(x0)
        o_ref[0:1, :] = x0[0:1, :].astype(o_ref.dtype)

        def kbody(g, carry):
            cp_k(1, g).wait()

            def tbody(c, carry2):
                for t in range(TB):
                    r0 = pl.multiple_of((c * TB + t) * 128, 128)
                    k0buf[g, pl.ds(r0, 128), :] = k1buf[g, pl.ds(r0, 128), :].T
                return carry2
            lax.fori_loop(0, NT // TB, tbody, 0)
            ktf[g] = k0buf[g, (NT - XVMAX) * 128:, :].astype(f32)
            qg = q_sc[1, g]
            s = jnp.concatenate([jnp.dot(qg, k0buf[g, t * 128:(t + 1) * 128, :], preferred_element_type=f32)
                                 for t in range(NT)], axis=1)
            p, l = softmax(s)
            p_sc[g] = p
            l_sc[g] = jnp.broadcast_to(1.0 / l, (8, DH))
            return carry
        lax.fori_loop(0, HKV, kbody, 0)

        y_sc[...] = jnp.zeros((8, D), f32)

        def vbody(g, carry):
            cp_v(1, g).wait()
            o = jnp.dot(p_sc[g], vbuf[1, g], preferred_element_type=f32) * l_sc[g]
            y_sc[...] += wo_mxu(o_expand(o), g)
            return carry
        lax.fori_loop(0, HKV - 1, vbody, 0)
        g = HKV - 1
        o = jnp.zeros((8, DH), f32)
        for c in range(len(LASTP)):
            t0 = sum(LASTP[:c])
            t1 = t0 + LASTP[c]
            cp_vlast(c).wait()
            o = o + jnp.dot(p_sc[g, :, t0 * 128:t1 * 128], vbuf[1, g, t0 * 128:t1 * 128, :],
                            preferred_element_type=f32)
        o_sc[...] = o

    pl.run_scoped(streamed, pltpu.SemaphoreType.DMA((NSEM,)))

    zmask = jnp.full((8, 128), z_sc[0], jnp.int32).astype(u32)
    k_u = k0buf.bitcast(u32)
    v_u = vbuf.bitcast(u32)
    g = HKV - 1
    x1 = jnp.broadcast_to(xbuf[...].astype(f32)[1:2, :], (8, D))
    o = o_sc[...] * l_sc[g]
    y = y_sc[...] + wo_mxu(o_expand(o), g)
    m = jnp.mean(x1, axis=-1, keepdims=True)
    x1 = x1 + rowsum(y)
    x1, m = ffn_fast(x1, m, zmask)
    xb, xf = _rnd(x1)
    m, rs = _stats1(xf, m)
    csc = rs * (SCALE * LOG2E)
    qs = [None] * HKV
    res = []
    clock = [0]
    zdep = {}
    qpk = {}

    def tied(v):
        i = (clock[0] - LAG) // TG * TG
        if i < 0:
            return v
        if i not in zdep:
            zdep[i] = pltpu.bitcast(res[i], u32) & zmask
        return pltpu.bitcast(pltpu.bitcast(v, u32) | zdep[i], f32)

    for g in range(QMXU):
        qs[g] = _rnd(q_raw_mxu(xb, m, g))[1]
    for c in range(ND):
        hb_sc[c * 128:(c + 1) * 128, :] = colb(xf[0:1, c * 128:(c + 1) * 128])

    def q_task(g):
        acc = [None] * REP
        for kb in range(D // 8):
            hv = tied(hb_sc[kb * 8:(kb + 1) * 8, :])
            for r in range(REP):
                acc[r] = _acc(acc[r], wqf[g * REP + r, kb * 8:(kb + 1) * 8, :] * hv)
            yield list(acc)
        qs[g] = _rnd(fold4(acc) - m * cq[g])[1]
        if XV[g]:
            for r in range(REP):
                qb_sc[g][r] = colb(qs[g][ROWS[r]:ROWS[r] + 1, :])

    yacc = [None] * ND

    def o_task(g):
        for r in range(REP):
            for kb in range(DH // 8):
                ov = tied(ob_sc[g][r, kb * 8:(kb + 1) * 8, :])
                for n in range(ND):
                    yacc[n] = _acc(yacc[n], wof[g * REP + r, kb * 8:(kb + 1) * 8, n * 128:(n + 1) * 128] * ov)
                yield list(yacc)

    def cb_task(g):
        for r in range(REP):
            yield [ob_sc[g][r, DH - 8:DH, :]]

    ss = [[None] * NT for _ in range(HKV)]
    ps = [None] * HKV
    ls = [None] * HKV

    def qb_task(g):
        for r in range(REP):
            yield [qb_sc[g][r, DH - 8:DH, :]]

    def kq_task(g):
        for bt in range(XV[g] // XT):
            tiles = [NT - XV[g] + bt * XT + i for i in range(XT)]
            acc = [[None] * REP for _ in range(XT)]
            for v in range(DH // 8):
                r0 = [(t - (NT - XVMAX)) * 128 + v * 8 for t in tiles]
                kv = [tied(ktf[g, r:r + 8, :]) for r in r0]
                for r in range(REP):
                    qv = qb_sc[g][r, v * 8:(v + 1) * 8, :]
                    for i in range(XT):
                        acc[i][r] = _acc(acc[i][r], kv[i] * qv)
                yield [a for al in acc for a in al]
            for i in range(XT):
                ss[g][tiles[i]] = fold4(acc[i])

    def sm_task(g):
        s = ss[g]
        mx = s[0]
        for t in range(1, NT):
            mx = jnp.maximum(mx, s[t])
        mx = jnp.broadcast_to(jnp.max(mx, axis=1, keepdims=True), (8, 128))
        out = []
        lacc = None
        for t0 in range(0, NT, SMG):
            mxt = tied(mx)
            es = [jnp.exp2((s[t] - mxt) * csc) for t in range(t0, t0 + SMG)]
            out += es
            while len(es) > 1:
                es = [es[i] + es[i + 1] for i in range(0, len(es), 2)]
            lacc = _acc(lacc, es[0])
            yield [lacc]
        ps[g] = out
        ls[g] = jnp.sum(lacc, axis=1, keepdims=True)

    stages = [("qk", 0)]
    for g in range(HKV):
        if g + 1 < HKV:
            stages.append(("qk", g + 1))
        stages.append(("pv", g))
    start, end = {}, {}
    tau = 0
    for st in stages:
        start[st] = tau
        tau += NT - XV[st[1]] if st[0] == "qk" else NT
        end[st] = tau

    tasks = []
    for g in range(QMXU, HKV):
        t0, t1 = (Q1A, Q1B) if g == 1 else (start[("qk", g - 1)], end[("qk", g - 1)])
        tasks.append([q_task(g), D // 8, t0, t1, 0, None])
    for g in range(HKV - 2):
        tasks.append([cb_task(g), REP, start[("pv", g + 1)] + CBA, start[("pv", g + 1)] + CBB, 0, None])
        tasks.append([o_task(g), REP * DH // 8, start[("pv", g + 1)], end[("pv", g + 1)], 0, None])
    tasks.append([o_task(HKV - 2), REP * DH // 8, end[("pv", HKV - 1)] - O6A, end[("pv", HKV - 1)] + O6B, 0, None])
    for g in range(HKV):
        if XV[g]:
            t1 = end[("pv", g - 1)] if g + 1 < HKV else end[("qk", g)] + 8
            tasks.append([qb_task(g), REP, start[("qk", g)] - 20, start[("qk", g)] - 4, 0, None])
            tasks.append([kq_task(g), XV[g] // XT * 16, start[("qk", g)], t1, 0, None])
    for g in range(HKV):
        st = ("qk", g + 1) if g + 1 < HKV else ("pv", g - 1)
        tasks.append([sm_task(g), NT // SMG, end[st] - SMA, end[st] - SMB, 0, None])

    def pinned(lhs, key=None):
        tau = clock[0]
        bits = None
        for tk in tasks:
            gen, n, t0, t1, done = tk[:5]
            if tau < t0 or done > n:
                continue
            want = n + 1 if tau >= t1 else (n * (tau - t0 + 1)) // (t1 - t0)
            while tk[4] < want:
                pin = next(gen, None)
                tk[4] += 1
                if pin is not None:
                    tk[5] = pin
            if tau % PG == PG - 1 and tk[5] is not None:
                pin = tk[5][(tau // PG) % len(tk[5])]
                tk[5] = None
                pb = pltpu.bitcast(pin, u32)
                bits = pb if bits is None else bits | pb
        clock[0] += 1
        if bits is not None:
            return pltpu.bitcast(pltpu.bitcast(lhs, u32) | (bits & zmask), f32).astype(bf16)
        if key is None:
            return lhs.astype(bf16)
        if key not in qpk:
            qpk[key] = lhs.astype(bf16)
        return qpk[key]

    for kind, g in stages:
        if kind == "qk":
            for t in range(NT - XV[g]):
                ss[g][t] = mm(pinned(qs[g], g), k_u[g, t * 64:(t + 1) * 64, :])
                res.append(ss[g][t])
        else:
            acc = [None] * 4
            for t in range(NT):
                d = mm(pinned(ps[g][t]), v_u[1, g, t * 64:(t + 1) * 64, :])
                res.append(d)
                acc[t % 4] = _acc(acc[t % 4], d)
            o = ((acc[0] + acc[1]) + (acc[2] + acc[3])) / ls[g]
            if g < HKV - 1:
                ob16 = _rnd(o)[1]
                for r in range(REP):
                    ob_sc[g][r] = colb(ob16[ROWS[r]:ROWS[r] + 1, :])
    clock[0] += O6L
    for tk in tasks:
        for _ in tk[0]:
            pass
    y = jnp.concatenate(yacc, axis=1) + wo_mxu(o_expand(o), HKV - 1)
    x1 = xf + rowsum(y)
    x1, _ = ffn_fast(x1, m, zmask)
    o_ref[1:2, :] = x1[0:1, :].astype(o_ref.dtype)


@jax.jit
def pallas_interleave_layers__gqa_block_cached__dense_activation_silu__decode_kernel(A_x, A_k_cache, A_v_cache, A_wq, A_wo, B_x, B_w1, B_w2):
    x2 = A_x.reshape(B, D)
    any_spec = pl.BlockSpec(memory_space=pl.ANY)
    out = pl.pallas_call(
        _kernel,
        out_shape=jax.ShapeDtypeStruct((B, D), bf16),
        in_specs=[any_spec] * 7,
        out_specs=pl.BlockSpec(memory_space=pltpu.VMEM),
        scratch_shapes=[
            pltpu.VMEM((B, D), bf16),
            pltpu.VMEM((HKV, SK, DH), bf16),
            pltpu.VMEM((HKV, SK, DH), bf16),
            pltpu.VMEM((B, HKV, SK, DH), bf16),
            pltpu.VMEM((D, HQ * DH), bf16),
            pltpu.VMEM((HQ * DH, D), bf16),
            pltpu.VMEM((D, F), bf16),
            pltpu.VMEM((F, D), bf16),
            pltpu.VMEM((HQ, D // 2, 128), u32),
            pltpu.VMEM((ND, HQ * DH // 2, 128), u32),
            pltpu.VMEM((NJ, D // 2, 128), u32),
            pltpu.VMEM((ND, F // 2, 128), u32),
            pltpu.VMEM((HQ, D, 128), f32),
            pltpu.VMEM((HQ, DH, D), f32),
            pltpu.VMEM((HV * 128, D), f32),
            pltpu.VMEM((HV * 128, D), f32),
            pltpu.VMEM((HKV, 8, DH), f32),
            pltpu.VMEM((8, F), f32),
            pltpu.VMEM((B, HKV, 8, DH), bf16),
            pltpu.VMEM((HKV, 8, SK), bf16),
            pltpu.VMEM((HKV, 8, DH), f32),
            pltpu.VMEM((8, D), f32),
            pltpu.VMEM((8, DH), f32),
            pltpu.VMEM((D, 128), f32),
            pltpu.SMEM((1,), jnp.int32),
            pltpu.VMEM((HKV, XVMAX * 128, 128), f32),
        ] + [pltpu.VMEM((REP, DH, 128), f32)] * (2 * HKV - 1),
        compiler_params=pltpu.CompilerParams(vmem_limit_bytes=124 * 1024 * 1024),
    )(x2, A_k_cache, A_v_cache, A_wq, A_wo, B_w1, B_w2)
    return out.reshape(B, 1, D)
```

```python
import jax
import jax.numpy as jnp
from jax import lax
import jax.experimental.pallas as pl
import jax.experimental.pallas.tpu as pltpu

B, D = 2, 512
HQ, HKV, SK, DH = 32, 8, 8192, 128
REP = HQ // HKV
GW = REP * DH
F = 1792
EPS = 1e-5
SCALE = DH ** -0.5
LOG2E = 1.4426950408889634
NT = SK // 128
ND = D // 128
NJ = F // 128
bf16 = jnp.bfloat16
f32 = jnp.float32
u32 = jnp.uint32

ROWS = (3, 7, 1, 5)
LASTP = (32, 16, 8, 4, 4)
TB = 32
QMXU = 1
HV = 6
PJ = 6
LAG = 26
SMG = 4
Q1A, Q1B = 36, 58
SMA, SMB = 32, 2
XA, XB = 4, 4
XV = (0, 0, XA, XA, XA, XA, XA, XB)
XT = 2
XVMAX = max(max(XV), 1)
TG, PG = 4, 2
CBA, CBB = 0, 24
O6A, O6B, O6L = 4, 28, 8


def _stats(x):
    m = jnp.mean(x, axis=-1, keepdims=True)
    xc = x - m
    v = jnp.mean(xc * xc, axis=-1, keepdims=True)
    return m, lax.rsqrt(v + EPS)


def _stats1(x, c):
    d = x - c
    s1 = jnp.mean(d, axis=-1, keepdims=True)
    s2 = jnp.mean(d * d, axis=-1, keepdims=True)
    v = jnp.maximum(s2 - s1 * s1, 0.0)
    return c + s1, lax.rsqrt(v + EPS)


def _silu_half(h):
    return h + h * jnp.tanh(h)


def _rnd(x):
    xb = x.astype(bf16)
    return xb, xb.astype(f32)


def _acc(a, t):
    return t if a is None else a + t


def _kernel(x_hbm, k_hbm, v_hbm, wq_hbm, wo_hbm, w1_hbm, w2_hbm, o_ref,
            xbuf, k0buf, k1buf, vbuf, wq, wo, w1, w2,
            wqt, wot, w1t, w2t, wqf, wof, w1f, w2f, cq, c1,
            q_sc, p_sc, l_sc, y_sc, o_sc, hb_sc, z_sc, ktf, *bsc):
    ob_sc = bsc[:HKV - 1]
    qb_sc = bsc[HKV - 1:]
    z_sc[0] = 0
    row = lax.broadcasted_iota(jnp.int32, (8, DH), 0)

    def as_bf(x):
        return pltpu.bitcast(x, bf16)

    def mm(a, w_u32):
        return jnp.dot(a, as_bf(w_u32), preferred_element_type=f32)

    def pick_rows(parts):
        qg = parts[0]
        for r in range(1, REP):
            qg = jnp.where(row == ROWS[r], parts[r], qg)
        return qg

    def fold4(acc):
        a = [x + pltpu.roll(x, 4, 0) for x in acc]
        b01 = jnp.where(row < 4, a[0], a[1])
        b23 = jnp.where(row < 4, a[2], a[3])
        c01 = b01 + pltpu.roll(b01, 2, 0)
        c23 = b23 + pltpu.roll(b23, 6, 0)
        d = jnp.where((row & 2) == 2, c01, c23)
        return d + pltpu.roll(d, 1, 0)

    def q_raw_mxu(xb, m, g):
        return pick_rows([mm(xb, wqt[g * REP + r]) for r in range(REP)]) - m * cq[g]

    def softmax(s):
        m = jnp.max(s, axis=1, keepdims=True)
        p = jnp.exp(s - m)
        l = jnp.sum(p, axis=1, keepdims=True)
        return p.astype(bf16), l

    def o_expand(o):
        return jnp.concatenate([jnp.where(row == ROWS[r], o, 0.0).astype(bf16) for r in range(REP)], axis=1)

    def rowsum(y):
        return jnp.broadcast_to(jnp.sum(y, axis=0, keepdims=True), (8, D))

    def wo_mxu(oe, g):
        return jnp.concatenate([mm(oe, wot[n, pl.ds(g * (GW // 2), GW // 2), :]) for n in range(ND)], axis=1)

    def wo_last(o):
        y = [None] * ND
        for r in range(REP):
            oe = jnp.where(row == ROWS[r], o, 0.0).astype(bf16)
            r0 = ((HKV - 1) * REP + r) * 64
            for n in range(ND):
                y[n] = _acc(y[n], mm(oe, wot[n, r0:r0 + 64, :]))
        return jnp.concatenate(y, axis=1)

    def ffn(x):
        xb, xf = _rnd(x)
        m, rs = _stats(xf)
        a = jnp.concatenate([mm(xb, w1t[j]) for j in range(NJ)], axis=1)
        a = (a - m * c1[...]) * rs
        a = (a * jax.nn.sigmoid(a)).astype(bf16)
        return xf + jnp.concatenate([mm(a, w2t[n]) for n in range(ND)], axis=1)

    def colb(v):
        return jnp.broadcast_to(v, (128, 128)).T

    def after(v, dep, zmask):
        return pltpu.bitcast(pltpu.bitcast(v, u32) | (pltpu.bitcast(dep, u32) & zmask), f32)

    def ffn_fast(x, c, zmask):
        xb, xf = _rnd(x)
        m, rs = _stats1(xf, c)
        rs = rs * 0.5
        NM = NJ - HV
        x0p = after(xf[:, 0:128], jnp.broadcast_to(rs, (8, 128)), zmask)
        xbp = jnp.concatenate([x0p.astype(bf16), xb[:, 128:]], axis=1)
        pre = [mm(xb if j < PJ else xbp, w1t[j]) for j in range(NM)]
        yv = [None] * ND
        for rb in range(HV * 16):
            acc = None
            for c_ in range(ND):
                acc = _acc(acc, w1f[rb * 8:(rb + 1) * 8, c_ * 128:(c_ + 1) * 128] * xf[:, c_ * 128:(c_ + 1) * 128])
            a = jnp.broadcast_to(jnp.sum(acc, axis=1, keepdims=True), (8, 128))
            a = _silu_half(a * rs)
            for n in range(ND):
                yv[n] = _acc(yv[n], w2f[rb * 8:(rb + 1) * 8, n * 128:(n + 1) * 128] * a)
        y = [None] * ND
        for j in range(NM):
            a = (pre[j] - m * c1[:, j * 128:(j + 1) * 128]) * rs
            a = _silu_half(a).astype(bf16)
            for n in range(ND):
                y[n] = _acc(y[n], mm(a, w2t[n, j * 64:(j + 1) * 64, :]))
        xf = xf + rowsum(jnp.concatenate(yv, axis=1))
        return xf + jnp.concatenate(y, axis=1), m

    NSEM = 5 + 2 * B * HKV + len(LASTP)

    def streamed(sem):
        cp_x = pltpu.make_async_copy(x_hbm, xbuf, sem.at[0])
        cp_wq = pltpu.make_async_copy(wq_hbm, wq, sem.at[1])
        cp_wo = pltpu.make_async_copy(wo_hbm, wo, sem.at[2])
        cp_w1 = pltpu.make_async_copy(w1_hbm, w1, sem.at[3])
        cp_w2 = pltpu.make_async_copy(w2_hbm, w2, sem.at[4])

        def cp_k(b, g):
            return pltpu.make_async_copy(k_hbm.at[b, g], (k0buf, k1buf)[b].at[g], sem.at[5 + (b * HKV + g) * 2])

        def cp_v(b, g):
            return pltpu.make_async_copy(v_hbm.at[b, g], vbuf.at[b, g], sem.at[6 + (b * HKV + g) * 2])

        def cp_vlast(c):
            r0 = sum(LASTP[:c]) * 128
            n = LASTP[c] * 128
            return pltpu.make_async_copy(v_hbm.at[1, HKV - 1, pl.ds(r0, n)],
                                         vbuf.at[1, HKV - 1, pl.ds(r0, n)],
                                         sem.at[5 + 2 * B * HKV + c])

        cp_wq.start()
        cp_x.start()
        for g in range(HKV):
            cp_k(0, g).start()
            cp_v(0, g).start()
        cp_wo.start()
        cp_w1.start()
        cp_w2.start()
        for g in range(HKV):
            cp_k(1, g).start()
        for g in range(HKV - 1):
            cp_v(1, g).start()
        for c in range(len(LASTP)):
            cp_vlast(c).start()

        ones = jnp.ones((8, D), bf16)

        def compute_q(x, slot):
            xb, xf = _rnd(x)
            m, rs = _stats(xf)
            for g in range(HKV):
                q_sc[slot, g] = (q_raw_mxu(xb, m, g) * (rs * SCALE)).astype(bf16)

        def attention0(wait):
            def body(g, carry):
                if wait:
                    cp_k(0, g).wait()
                s = lax.dot_general(q_sc[0, g], k0buf[g], (((1,), (1,)), ((), ())),
                                    preferred_element_type=f32)
                p, l = softmax(s)
                if wait:
                    cp_v(0, g).wait()
                o = jnp.dot(p, vbuf[0, g], preferred_element_type=f32) / l
                p_sc[g, :, 0:GW] = o_expand(o)
                return carry
            lax.fori_loop(0, HKV, body, 0)

        def out_proj0():
            ofull = jnp.concatenate([p_sc[g, :, 0:GW] for g in range(HKV)], axis=1)
            return rowsum(jnp.dot(ofull, wo[...], preferred_element_type=f32))

        cp_x.wait()
        cp_wq.wait()
        xs = xbuf[...].astype(f32)
        x0 = jnp.broadcast_to(xs[0:1, :], (8, D))
        x1 = jnp.broadcast_to(xs[1:2, :], (8, D))

        def prep_q(j, carry):
            w = wq[:, pl.ds(pl.multiple_of(j * 128, 128), 128)]
            wqt[j] = pltpu.bitcast(w, u32)
            wqf[j] = w.astype(f32)
            return carry
        lax.fori_loop(0, HQ, prep_q, 0)
        for g in range(HKV):
            cq[g] = pick_rows([mm(ones, wqt[g * REP + r]) for r in range(REP)])
        compute_q(x0, 0)
        compute_q(x1, 1)
        attention0(True)
        cp_wo.wait()
        x0 = x0 + out_proj0()

        def prep_o(i, carry):
            w = wo[pl.ds(pl.multiple_of(i * 128, 128), 128), :]
            wof[i] = w.astype(f32)
            for n in range(ND):
                wot[n, pl.ds(pl.multiple_of(i * 64, 64), 64), :] = pltpu.bitcast(w[:, n * 128:(n + 1) * 128], u32)
            return carry
        lax.fori_loop(0, HQ, prep_o, 0)
        cp_w1.wait()
        cp_w2.wait()
        for j in range(NJ):
            w1t[j] = pltpu.bitcast(w1[:, j * 128:(j + 1) * 128], u32)
        for n in range(ND):
            w2t[n] = pltpu.bitcast(w2[:, n * 128:(n + 1) * 128], u32)
        c1[...] = jnp.dot(ones, w1[...], preferred_element_type=f32)
        for r in range(HV):
            j = NJ - HV + r
            w1f[r * 128:(r + 1) * 128, :] = (w1[:, j * 128:(j + 1) * 128].astype(f32)
                                             - c1[0:1, j * 128:(j + 1) * 128] * (1.0 / D)).T
            w2f[r * 128:(r + 1) * 128, :] = w2[j * 128:(j + 1) * 128, :].astype(f32)
        x0 = ffn(x0)
        compute_q(x0, 0)
        attention0(False)
        x0 = _rnd(x0)[1] + out_proj0()
        x0 = ffn(x0)
        o_ref[0:1, :] = x0[0:1, :].astype(o_ref.dtype)

        def kbody(g, carry):
            cp_k(1, g).wait()

            def tbody(c, carry2):
                for t in range(TB):
                    r0 = pl.multiple_of((c * TB + t) * 128, 128)
                    k0buf[g, pl.ds(r0, 128), :] = k1buf[g, pl.ds(r0, 128), :].T
                return carry2
            lax.fori_loop(0, NT // TB, tbody, 0)
            ktf[g] = k0buf[g, (NT - XVMAX) * 128:, :].astype(f32)
            qg = q_sc[1, g]
            s = jnp.concatenate([jnp.dot(qg, k0buf[g, t * 128:(t + 1) * 128, :], preferred_element_type=f32)
                                 for t in range(NT)], axis=1)
            p, l = softmax(s)
            p_sc[g] = p
            l_sc[g] = jnp.broadcast_to(1.0 / l, (8, DH))
            return carry
        lax.fori_loop(0, HKV, kbody, 0)

        y_sc[...] = jnp.zeros((8, D), f32)

        def vbody(g, carry):
            cp_v(1, g).wait()
            o = jnp.dot(p_sc[g], vbuf[1, g], preferred_element_type=f32) * l_sc[g]
            y_sc[...] += wo_mxu(o_expand(o), g)
            return carry
        lax.fori_loop(0, HKV - 1, vbody, 0)
        g = HKV - 1
        o = jnp.zeros((8, DH), f32)
        for c in range(len(LASTP)):
            t0 = sum(LASTP[:c])
            t1 = t0 + LASTP[c]
            cp_vlast(c).wait()
            o = o + jnp.dot(p_sc[g, :, t0 * 128:t1 * 128], vbuf[1, g, t0 * 128:t1 * 128, :],
                            preferred_element_type=f32)
        o_sc[...] = o

    pl.run_scoped(streamed, pltpu.SemaphoreType.DMA((NSEM,)))

    zmask = jnp.full((8, 128), z_sc[0], jnp.int32).astype(u32)
    k_u = k0buf.bitcast(u32)
    v_u = vbuf.bitcast(u32)
    g = HKV - 1
    x1 = jnp.broadcast_to(xbuf[...].astype(f32)[1:2, :], (8, D))
    o = o_sc[...] * l_sc[g]
    y = y_sc[...] + wo_last(o)
    m = jnp.mean(x1, axis=-1, keepdims=True)
    x1 = x1 + rowsum(y)
    x1, m = ffn_fast(x1, m, zmask)
    xb, xf = _rnd(x1)
    m, rs = _stats1(xf, m)
    csc = rs * (SCALE * LOG2E)
    qs = [None] * HKV
    res = []
    clock = [0]
    zdep = {}
    qpk = {}

    def tied(v):
        i = (clock[0] - LAG) // TG * TG
        if i < 0:
            return v
        if i not in zdep:
            zdep[i] = pltpu.bitcast(res[i], u32) & zmask
        return pltpu.bitcast(pltpu.bitcast(v, u32) | zdep[i], f32)

    for g in range(QMXU):
        qs[g] = _rnd(q_raw_mxu(xb, m, g))[1]
    for c in range(ND):
        hb_sc[c * 128:(c + 1) * 128, :] = colb(xf[0:1, c * 128:(c + 1) * 128])

    def q_task(g):
        acc = [None] * REP
        for kb in range(D // 8):
            hv = tied(hb_sc[kb * 8:(kb + 1) * 8, :])
            for r in range(REP):
                acc[r] = _acc(acc[r], wqf[g * REP + r, kb * 8:(kb + 1) * 8, :] * hv)
            yield list(acc)
        qs[g] = _rnd(fold4(acc) - m * cq[g])[1]
        if XV[g]:
            for r in range(REP):
                qb_sc[g][r] = colb(qs[g][ROWS[r]:ROWS[r] + 1, :])

    yacc = [None] * ND

    def o_task(g):
        for r in range(REP):
            for kb in range(DH // 8):
                ov = tied(ob_sc[g][r, kb * 8:(kb + 1) * 8, :])
                for n in range(ND):
                    yacc[n] = _acc(yacc[n], wof[g * REP + r, kb * 8:(kb + 1) * 8, n * 128:(n + 1) * 128] * ov)
                yield list(yacc)

    def cb_task(g):
        for r in range(REP):
            yield [ob_sc[g][r, DH - 8:DH, :]]

    ss = [[None] * NT for _ in range(HKV)]
    ps = [None] * HKV
    ls = [None] * HKV

    def qb_task(g):
        for r in range(REP):
            yield [qb_sc[g][r, DH - 8:DH, :]]

    def kq_task(g):
        for bt in range(XV[g] // XT):
            tiles = [NT - XV[g] + bt * XT + i for i in range(XT)]
            acc = [[None] * REP for _ in range(XT)]
            for v in range(DH // 8):
                r0 = [(t - (NT - XVMAX)) * 128 + v * 8 for t in tiles]
                kv = [tied(ktf[g, r:r + 8, :]) for r in r0]
                for r in range(REP):
                    qv = qb_sc[g][r, v * 8:(v + 1) * 8, :]
                    for i in range(XT):
                        acc[i][r] = _acc(acc[i][r], kv[i] * qv)
                yield [a for al in acc for a in al]
            for i in range(XT):
                ss[g][tiles[i]] = fold4(acc[i])

    def sm_task(g):
        s = ss[g]
        mx = s[0]
        for t in range(1, NT):
            mx = jnp.maximum(mx, s[t])
        mx = jnp.broadcast_to(jnp.max(mx, axis=1, keepdims=True), (8, 128))
        out = []
        lacc = None
        for t0 in range(0, NT, SMG):
            mxt = tied(mx)
            es = [jnp.exp2((s[t] - mxt) * csc) for t in range(t0, t0 + SMG)]
            out += es
            while len(es) > 1:
                es = [es[i] + es[i + 1] for i in range(0, len(es), 2)]
            lacc = _acc(lacc, es[0])
            yield [lacc]
        ps[g] = out
        ls[g] = jnp.sum(lacc, axis=1, keepdims=True)

    stages = [("qk", 0)]
    for g in range(HKV):
        if g + 1 < HKV:
            stages.append(("qk", g + 1))
        stages.append(("pv", g))
    start, end = {}, {}
    tau = 0
    for st in stages:
        start[st] = tau
        tau += NT - XV[st[1]] if st[0] == "qk" else NT
        end[st] = tau

    tasks = []
    for g in range(QMXU, HKV):
        t0, t1 = (Q1A, Q1B) if g == 1 else (start[("qk", g - 1)], end[("qk", g - 1)])
        tasks.append([q_task(g), D // 8, t0, t1, 0, None])
    for g in range(HKV - 2):
        tasks.append([cb_task(g), REP, start[("pv", g + 1)] + CBA, start[("pv", g + 1)] + CBB, 0, None])
        tasks.append([o_task(g), REP * DH // 8, start[("pv", g + 1)], end[("pv", g + 1)], 0, None])
    tasks.append([o_task(HKV - 2), REP * DH // 8, end[("pv", HKV - 1)] - O6A, end[("pv", HKV - 1)] + O6B, 0, None])
    for g in range(HKV):
        if XV[g]:
            t1 = end[("pv", g - 1)] if g + 1 < HKV else end[("qk", g)] + 8
            tasks.append([qb_task(g), REP, start[("qk", g)] - 20, start[("qk", g)] - 4, 0, None])
            tasks.append([kq_task(g), XV[g] // XT * 16, start[("qk", g)], t1, 0, None])
    for g in range(HKV):
        st = ("qk", g + 1) if g + 1 < HKV else ("pv", g - 1)
        tasks.append([sm_task(g), NT // SMG, end[st] - SMA, end[st] - SMB, 0, None])

    def pinned(lhs, key=None):
        tau = clock[0]
        bits = None
        for tk in tasks:
            gen, n, t0, t1, done = tk[:5]
            if tau < t0 or done > n:
                continue
            want = n + 1 if tau >= t1 else (n * (tau - t0 + 1)) // (t1 - t0)
            while tk[4] < want:
                pin = next(gen, None)
                tk[4] += 1
                if pin is not None:
                    tk[5] = pin
            if tau % PG == PG - 1 and tk[5] is not None:
                pin = tk[5][(tau // PG) % len(tk[5])]
                tk[5] = None
                pb = pltpu.bitcast(pin, u32)
                bits = pb if bits is None else bits | pb
        clock[0] += 1
        if bits is not None:
            return pltpu.bitcast(pltpu.bitcast(lhs, u32) | (bits & zmask), f32).astype(bf16)
        if key is None:
            return lhs.astype(bf16)
        if key not in qpk:
            qpk[key] = lhs.astype(bf16)
        return qpk[key]

    for kind, g in stages:
        if kind == "qk":
            for t in range(NT - XV[g]):
                ss[g][t] = mm(pinned(qs[g], g), k_u[g, t * 64:(t + 1) * 64, :])
                res.append(ss[g][t])
        else:
            acc = [None] * 4
            for t in range(NT):
                d = mm(pinned(ps[g][t]), v_u[1, g, t * 64:(t + 1) * 64, :])
                res.append(d)
                acc[t % 4] = _acc(acc[t % 4], d)
            o = ((acc[0] + acc[1]) + (acc[2] + acc[3])) / ls[g]
            if g < HKV - 1:
                ob16 = _rnd(o)[1]
                for r in range(REP):
                    ob_sc[g][r] = colb(ob16[ROWS[r]:ROWS[r] + 1, :])
    clock[0] += O6L
    for tk in tasks:
        for _ in tk[0]:
            pass
    y = jnp.concatenate(yacc, axis=1) + wo_last(o)
    x1 = xf + rowsum(y)
    x1, _ = ffn_fast(x1, m, zmask)
    o_ref[1:2, :] = x1[0:1, :].astype(o_ref.dtype)


@jax.jit
def pallas_interleave_layers__gqa_block_cached__dense_activation_silu__decode_kernel(A_x, A_k_cache, A_v_cache, A_wq, A_wo, B_x, B_w1, B_w2):
    x2 = A_x.reshape(B, D)
    any_spec = pl.BlockSpec(memory_space=pl.ANY)
    out = pl.pallas_call(
        _kernel,
        out_shape=jax.ShapeDtypeStruct((B, D), bf16),
        in_specs=[any_spec] * 7,
        out_specs=pl.BlockSpec(memory_space=pltpu.VMEM),
        scratch_shapes=[
            pltpu.VMEM((B, D), bf16),
            pltpu.VMEM((HKV, SK, DH), bf16),
            pltpu.VMEM((HKV, SK, DH), bf16),
            pltpu.VMEM((B, HKV, SK, DH), bf16),
            pltpu.VMEM((D, HQ * DH), bf16),
            pltpu.VMEM((HQ * DH, D), bf16),
            pltpu.VMEM((D, F), bf16),
            pltpu.VMEM((F, D), bf16),
            pltpu.VMEM((HQ, D // 2, 128), u32),
            pltpu.VMEM((ND, HQ * DH // 2, 128), u32),
            pltpu.VMEM((NJ, D // 2, 128), u32),
            pltpu.VMEM((ND, F // 2, 128), u32),
            pltpu.VMEM((HQ, D, 128), f32),
            pltpu.VMEM((HQ, DH, D), f32),
            pltpu.VMEM((HV * 128, D), f32),
            pltpu.VMEM((HV * 128, D), f32),
            pltpu.VMEM((HKV, 8, DH), f32),
            pltpu.VMEM((8, F), f32),
            pltpu.VMEM((B, HKV, 8, DH), bf16),
            pltpu.VMEM((HKV, 8, SK), bf16),
            pltpu.VMEM((HKV, 8, DH), f32),
            pltpu.VMEM((8, D), f32),
            pltpu.VMEM((8, DH), f32),
            pltpu.VMEM((D, 128), f32),
            pltpu.SMEM((1,), jnp.int32),
            pltpu.VMEM((HKV, XVMAX * 128, 128), f32),
        ] + [pltpu.VMEM((REP, DH, 128), f32)] * (2 * HKV - 1),
        compiler_params=pltpu.CompilerParams(vmem_limit_bytes=124 * 1024 * 1024),
    )(x2, A_k_cache, A_v_cache, A_wq, A_wo, B_w1, B_w2)
    return out.reshape(B, 1, D)
```

```python
import jax
import jax.numpy as jnp
from jax import lax
import jax.experimental.pallas as pl
import jax.experimental.pallas.tpu as pltpu

B, D = 2, 512
HQ, HKV, SK, DH = 32, 8, 8192, 128
REP = HQ // HKV
GW = REP * DH
F = 1792
EPS = 1e-5
SCALE = DH ** -0.5
LOG2E = 1.4426950408889634
NT = SK // 128
ND = D // 128
NJ = F // 128
bf16 = jnp.bfloat16
f32 = jnp.float32
u32 = jnp.uint32

ROWS = (3, 7, 1, 5)
LASTP = (32, 16, 8, 4, 4)
VPK = 56
TB = 32

QMXU = 1
HV = 6
PJ = 6
XV = (0, 0, 4, 4, 4, 4, 4, 4)
XT = 2
XVMAX = max(XV)
LAG = 26
TG, PG = 4, 2
SMG = 4
Q1A, Q1B = 36, 58
SMA, SMB = 32, 2
CBA, CBB = 0, 24
O6A, O6B, O6L = 4, 28, 8


def _stats(x):
    m = jnp.mean(x, axis=-1, keepdims=True)
    xc = x - m
    v = jnp.mean(xc * xc, axis=-1, keepdims=True)
    return m, lax.rsqrt(v + EPS)


def _stats1(x, c):
    d = x - c
    s1 = jnp.mean(d, axis=-1, keepdims=True)
    s2 = jnp.mean(d * d, axis=-1, keepdims=True)
    v = jnp.maximum(s2 - s1 * s1, 0.0)
    return c + s1, lax.rsqrt(v + EPS)


def _silu_half(h):
    return h + h * jnp.tanh(h)


def _rnd(x):
    xb = x.astype(bf16)
    return xb, xb.astype(f32)


def _acc(a, t):
    return t if a is None else a + t


def _kernel(x_hbm, k_hbm, v_hbm, wq_hbm, wo_hbm, w1_hbm, w2_hbm, o_ref,
            xbuf, k1buf, v1buf, wq, wo, w1, w2,
            wqt, wot, w1t, w2t, wqf, wof, w1f, w2f, cq, c1,
            q_sc, p_sc, l_sc, y_sc, hb_sc, z_sc, ktf, *bsc):
    ob_sc = bsc[:HKV - 1]
    qb_sc = bsc[HKV - 1:]
    z_sc[0] = 0
    row = lax.broadcasted_iota(jnp.int32, (8, DH), 0)

    def as_bf(x):
        return pltpu.bitcast(x, bf16)

    def mm(a, w_u32):
        return jnp.dot(a, as_bf(w_u32), preferred_element_type=f32)

    def pick_rows(parts):
        qg = parts[0]
        for r in range(1, REP):
            qg = jnp.where(row == ROWS[r], parts[r], qg)
        return qg

    def fold4(acc):
        a = [x + pltpu.roll(x, 4, 0) for x in acc]
        b01 = jnp.where(row < 4, a[0], a[1])
        b23 = jnp.where(row < 4, a[2], a[3])
        c01 = b01 + pltpu.roll(b01, 2, 0)
        c23 = b23 + pltpu.roll(b23, 6, 0)
        d = jnp.where((row & 2) == 2, c01, c23)
        return d + pltpu.roll(d, 1, 0)

    def q_raw_mxu(xb, m, g):
        return pick_rows([mm(xb, wqt[g * REP + r]) for r in range(REP)]) - m * cq[g]

    def softmax(s):
        m = jnp.max(s, axis=1, keepdims=True)
        p = jnp.exp(s - m)
        l = jnp.sum(p, axis=1, keepdims=True)
        return p.astype(bf16), l

    def o_expand(o):
        return jnp.concatenate([jnp.where(row == ROWS[r], o, 0.0).astype(bf16) for r in range(REP)], axis=1)

    def rowsum(y):
        return jnp.broadcast_to(jnp.sum(y, axis=0, keepdims=True), (8, D))

    def wo_mxu(oe, g):
        return jnp.concatenate([mm(oe, wot[n, pl.ds(g * (GW // 2), GW // 2), :]) for n in range(ND)], axis=1)

    def wo_last(o):
        y = [None] * ND
        for r in range(REP):
            oe = jnp.broadcast_to(o[ROWS[r]:ROWS[r] + 1, :], (8, DH)).astype(bf16)
            r0 = ((HKV - 1) * REP + r) * 64
            for n in range(ND):
                y[n] = _acc(y[n], mm(oe, wot[n, r0:r0 + 64, :]))
        return jnp.concatenate(y, axis=1)

    def ffn(x):
        xb, xf = _rnd(x)
        m, rs = _stats(xf)
        a = jnp.concatenate([mm(xb, w1t[j]) for j in range(NJ)], axis=1)
        a = (a - m * c1[...]) * rs
        a = (a * jax.nn.sigmoid(a)).astype(bf16)
        return xf + jnp.concatenate([mm(a, w2t[n]) for n in range(ND)], axis=1)

    def colb(v):
        return jnp.broadcast_to(v, (128, 128)).T

    def after(v, dep, zmask):
        return pltpu.bitcast(pltpu.bitcast(v, u32) | (pltpu.bitcast(dep, u32) & zmask), f32)

    def ffn_fast(x, c, zmask):
        xb, xf = _rnd(x)
        m, rs = _stats1(xf, c)
        rs = rs * 0.5
        NM = NJ - HV
        x0p = after(xf[:, 0:128], jnp.broadcast_to(rs, (8, 128)), zmask)
        xbp = jnp.concatenate([x0p.astype(bf16), xb[:, 128:]], axis=1)
        pre = [mm(xb if j < PJ else xbp, w1t[j]) for j in range(NM)]
        yv = [None] * ND
        for rb in range(HV * 16):
            acc = None
            for c_ in range(ND):
                acc = _acc(acc, w1f[rb * 8:(rb + 1) * 8, c_ * 128:(c_ + 1) * 128] * xf[:, c_ * 128:(c_ + 1) * 128])
            a = jnp.broadcast_to(jnp.sum(acc, axis=1, keepdims=True), (8, 128))
            a = _silu_half(a * rs)
            for n in range(ND):
                yv[n] = _acc(yv[n], w2f[rb * 8:(rb + 1) * 8, n * 128:(n + 1) * 128] * a)
        y = [None] * ND
        for j in range(NM):
            a = (pre[j] - m * c1[:, j * 128:(j + 1) * 128]) * rs
            a = _silu_half(a).astype(bf16)
            for n in range(ND):
                y[n] = _acc(y[n], mm(a, w2t[n, j * 64:(j + 1) * 64, :]))
        xf = xf + rowsum(jnp.concatenate(yv, axis=1))
        return xf + jnp.concatenate(y, axis=1), m

    NSEM = 5 + 2 * B * HKV + len(LASTP)

    def whole(sem):
        cp_x = pltpu.make_async_copy(x_hbm, xbuf, sem.at[0])
        cp_wq = pltpu.make_async_copy(wq_hbm, wq, sem.at[1])
        cp_wo = pltpu.make_async_copy(wo_hbm, wo, sem.at[2])
        cp_w1 = pltpu.make_async_copy(w1_hbm, w1, sem.at[3])
        cp_w2 = pltpu.make_async_copy(w2_hbm, w2, sem.at[4])

        def cp_k(b, g, dst):
            return pltpu.make_async_copy(k_hbm.at[b, g], dst.at[g], sem.at[5 + (b * HKV + g) * 2])

        def cp_v(b, g, dst):
            return pltpu.make_async_copy(v_hbm.at[b, g], dst.at[g], sem.at[6 + (b * HKV + g) * 2])

        def cp_vlast(c):
            r0 = sum(LASTP[:c]) * 128
            n = LASTP[c] * 128
            return pltpu.make_async_copy(v_hbm.at[1, HKV - 1, pl.ds(r0, n)],
                                         v1buf.at[HKV - 1, pl.ds(r0, n)],
                                         sem.at[5 + 2 * B * HKV + c])

        def batch0(k0buf, v0buf):
            cp_wq.start()
            cp_x.start()
            for g in range(HKV):
                cp_k(0, g, k0buf).start()
                cp_v(0, g, v0buf).start()
            cp_wo.start()
            cp_w1.start()
            cp_w2.start()
            for g in range(HKV):
                cp_k(1, g, k1buf).start()
            for g in range(HKV - 1):
                cp_v(1, g, v1buf).start()
            for c in range(len(LASTP)):
                cp_vlast(c).start()

            ones = jnp.ones((8, D), bf16)

            def compute_q(x, slot):
                xb, xf = _rnd(x)
                m, rs = _stats(xf)
                for g in range(HKV):
                    q_sc[slot, g] = (q_raw_mxu(xb, m, g) * (rs * SCALE)).astype(bf16)

            def attention0(wait):
                def body(g, carry):
                    if wait:
                        cp_k(0, g, k0buf).wait()
                    s = lax.dot_general(q_sc[0, g], k0buf[g], (((1,), (1,)), ((), ())),
                                        preferred_element_type=f32)
                    p, l = softmax(s)
                    if wait:
                        cp_v(0, g, v0buf).wait()
                    o = jnp.dot(p, v0buf[g], preferred_element_type=f32) / l
                    p_sc[g, :, 0:GW] = o_expand(o)
                    return carry
                lax.fori_loop(0, HKV, body, 0)

            def out_proj0():
                ofull = jnp.concatenate([p_sc[g, :, 0:GW] for g in range(HKV)], axis=1)
                return rowsum(jnp.dot(ofull, wo[...], preferred_element_type=f32))

            cp_x.wait()
            cp_wq.wait()
            xs = xbuf[...].astype(f32)
            x0 = jnp.broadcast_to(xs[0:1, :], (8, D))
            x1 = jnp.broadcast_to(xs[1:2, :], (8, D))

            def prep_q(j, carry):
                w = wq[:, pl.ds(pl.multiple_of(j * 128, 128), 128)]
                wqt[j] = pltpu.bitcast(w, u32)
                wqf[j] = w.astype(f32)
                return carry
            lax.fori_loop(0, HQ, prep_q, 0)
            for g in range(HKV):
                cq[g] = pick_rows([mm(ones, wqt[g * REP + r]) for r in range(REP)])
            compute_q(x0, 0)
            compute_q(x1, 1)
            attention0(True)
            cp_wo.wait()
            x0 = x0 + out_proj0()

            def prep_o(i, carry):
                w = wo[pl.ds(pl.multiple_of(i * 128, 128), 128), :]
                wof[i] = w.astype(f32)
                for n in range(ND):
                    wot[n, pl.ds(pl.multiple_of(i * 64, 64), 64), :] = pltpu.bitcast(w[:, n * 128:(n + 1) * 128], u32)
                return carry
            lax.fori_loop(0, HQ, prep_o, 0)
            cp_w1.wait()
            cp_w2.wait()
            for j in range(NJ):
                w1t[j] = pltpu.bitcast(w1[:, j * 128:(j + 1) * 128], u32)
            for n in range(ND):
                w2t[n] = pltpu.bitcast(w2[:, n * 128:(n + 1) * 128], u32)
            c1[...] = jnp.dot(ones, w1[...], preferred_element_type=f32)
            for r in range(HV):
                j = NJ - HV + r
                w1f[r * 128:(r + 1) * 128, :] = (w1[:, j * 128:(j + 1) * 128].astype(f32)
                                                 - c1[0:1, j * 128:(j + 1) * 128] * (1.0 / D)).T
                w2f[r * 128:(r + 1) * 128, :] = w2[j * 128:(j + 1) * 128, :].astype(f32)
            x0 = ffn(x0)
            compute_q(x0, 0)
            attention0(False)
            x0 = _rnd(x0)[1] + out_proj0()
            x0 = ffn(x0)
            o_ref[0:1, :] = x0[0:1, :].astype(o_ref.dtype)

        pl.run_scoped(batch0, pltpu.VMEM((HKV, SK, DH), bf16), pltpu.VMEM((HKV, SK, DH), bf16))

        def batch1(k_u, v_u):
            def kbody(g, carry):
                cp_k(1, g, k1buf).wait()

                def tbody(c, carry2):
                    for t in range(TB):
                        r0 = pl.multiple_of((c * TB + t) * 128, 128)
                        u0 = pl.multiple_of((c * TB + t) * 64, 64)
                        k_u[g, pl.ds(u0, 64), :] = pltpu.bitcast(k1buf[g, pl.ds(r0, 128), :].T, u32)
                    return carry2
                lax.fori_loop(0, NT // TB, tbody, 0)
                ktf[g] = as_bf(k_u[g, (NT - XVMAX) * 64:, :]).astype(f32)
                qg = q_sc[1, g]
                s = jnp.concatenate([mm(qg, k_u[g, t * 64:(t + 1) * 64, :]) for t in range(NT)], axis=1)
                p, l = softmax(s)
                p_sc[g] = p
                l_sc[g] = jnp.broadcast_to(1.0 / l, (8, DH))
                return carry
            lax.fori_loop(0, HKV, kbody, 0)

            y_sc[...] = jnp.zeros((8, D), f32)

            def vbody(g, carry):
                cp_v(1, g, v1buf).wait()
                v = v1buf[g]
                v_u[g] = pltpu.bitcast(v, u32)
                o = jnp.dot(p_sc[g], v, preferred_element_type=f32) * l_sc[g]
                y_sc[...] += wo_mxu(o_expand(o), g)
                return carry
            lax.fori_loop(0, HKV - 1, vbody, 0)
            g = HKV - 1
            o = jnp.zeros((8, DH), f32)
            for c in range(len(LASTP)):
                t0 = sum(LASTP[:c])
                t1 = t0 + LASTP[c]
                cp_vlast(c).wait()
                v = v1buf[g, t0 * 128:t1 * 128, :]
                if t1 <= VPK:
                    v_u[g, t0 * 64:t1 * 64, :] = pltpu.bitcast(v, u32)
                o = o + jnp.dot(p_sc[g, :, t0 * 128:t1 * 128], v, preferred_element_type=f32)

            zmask = jnp.full((8, 128), z_sc[0], jnp.int32).astype(u32)
            g = HKV - 1
            x1 = jnp.broadcast_to(xbuf[...].astype(f32)[1:2, :], (8, D))
            o = o * l_sc[g]
            m = jnp.mean(x1, axis=-1, keepdims=True)
            x1 = (x1 + rowsum(y_sc[...])) + wo_last(o)
            x1, m = ffn_fast(x1, m, zmask)
            xb, xf = _rnd(x1)
            m, rs = _stats1(xf, m)
            csc = rs * (SCALE * LOG2E)
            qs = [None] * HKV
            res = []
            clock = [0]
            zdep = {}
            qpk = {}

            def tied(v):
                i = (clock[0] - LAG) // TG * TG
                if i < 0:
                    return v
                if i not in zdep:
                    zdep[i] = pltpu.bitcast(res[i], u32) & zmask
                return pltpu.bitcast(pltpu.bitcast(v, u32) | zdep[i], f32)

            odd = (row & 1) == 1

            def set_q(g, q):
                qa = jnp.where(odd, _rnd(q)[1], 0.0)
                qs[g] = (qa, pltpu.roll(qa, 7, 0))
                if XV[g]:
                    for r in range(REP):
                        qb_sc[g][r] = colb(qa[ROWS[r]:ROWS[r] + 1, :])

            for g in range(QMXU):
                set_q(g, q_raw_mxu(xb, m, g))
            for c in range(ND):
                hb_sc[c * 128:(c + 1) * 128, :] = colb(xf[0:1, c * 128:(c + 1) * 128])

            def q_task(g):
                acc = [None] * REP
                for kb in range(D // 8):
                    hv = tied(hb_sc[kb * 8:(kb + 1) * 8, :])
                    for r in range(REP):
                        acc[r] = _acc(acc[r], wqf[g * REP + r, kb * 8:(kb + 1) * 8, :] * hv)
                    yield list(acc)
                set_q(g, fold4(acc) - m * cq[g])

            yacc = [None] * ND

            def o_task(g):
                for r in range(REP):
                    for kb in range(DH // 8):
                        ov = tied(ob_sc[g][r, kb * 8:(kb + 1) * 8, :])
                        for n in range(ND):
                            yacc[n] = _acc(yacc[n], wof[g * REP + r, kb * 8:(kb + 1) * 8, n * 128:(n + 1) * 128] * ov)
                        yield list(yacc)

            def cb_task(g):
                for r in range(REP):
                    yield [ob_sc[g][r, DH - 8:DH, :]]

            ss = [[None] * (NT // 2) for _ in range(HKV)]
            ps = [None] * HKV
            ls = [None] * HKV

            def qb_task(g):
                for r in range(REP):
                    yield [qb_sc[g][r, DH - 8:DH, :]]

            def kq_task(g):
                for bt in range(XV[g] // XT):
                    tiles = [NT - XV[g] + bt * XT + i for i in range(XT)]
                    acc = [[None] * REP for _ in range(XT)]
                    for v in range(DH // 8):
                        r0 = [(t - (NT - XVMAX)) * 128 + v * 8 for t in tiles]
                        kv = [tied(ktf[g, r:r + 8, :]) for r in r0]
                        for r in range(REP):
                            qv = qb_sc[g][r, v * 8:(v + 1) * 8, :]
                            for i in range(XT):
                                acc[i][r] = _acc(acc[i][r], kv[i] * qv)
                        yield [a for al in acc for a in al]
                    ss[g][tiles[0] // 2] = jnp.where(odd, fold4(acc[0]), pltpu.roll(fold4(acc[1]), 7, 0))

            def sm_task(g):
                s = ss[g]
                mx = s[0]
                for t in range(1, NT // 2):
                    mx = jnp.maximum(mx, s[t])
                mx = jnp.maximum(mx, jnp.where(odd, pltpu.roll(mx, 1, 0), pltpu.roll(mx, 7, 0)))
                mx = jnp.broadcast_to(jnp.max(mx, axis=1, keepdims=True), (8, 128))
                out = []
                lacc = None
                for t0 in range(0, NT // 2, SMG):
                    mxt = tied(mx)
                    es = [jnp.exp2((s[t] - mxt) * csc) for t in range(t0, t0 + SMG)]
                    out += es
                    while len(es) > 1:
                        es = [es[i] + es[i + 1] for i in range(0, len(es), 2)]
                    lacc = _acc(lacc, es[0])
                    yield [lacc]
                ps[g] = out
                ls[g] = jnp.sum(lacc + pltpu.roll(lacc, 1, 0), axis=1, keepdims=True)

            stages = [("qk", 0)]
            for g in range(HKV):
                if g + 1 < HKV:
                    stages.append(("qk", g + 1))
                stages.append(("pv", g))
            start, end = {}, {}
            tau = 0
            for st in stages:
                start[st] = tau
                tau += NT - XV[st[1]] if st[0] == "qk" else NT
                end[st] = tau

            tasks = []
            for g in range(QMXU, HKV):
                t0, t1 = (Q1A, Q1B) if g == 1 else (start[("qk", g - 1)], end[("qk", g - 1)])
                tasks.append([q_task(g), D // 8, t0, t1, 0, None])
            for g in range(HKV - 2):
                tasks.append([cb_task(g), REP, start[("pv", g + 1)] + CBA, start[("pv", g + 1)] + CBB, 0, None])
                tasks.append([o_task(g), REP * DH // 8, start[("pv", g + 1)], end[("pv", g + 1)], 0, None])
            tasks.append([o_task(HKV - 2), REP * DH // 8, end[("pv", HKV - 1)] - O6A, end[("pv", HKV - 1)] + O6B, 0, None])
            for g in range(HKV):
                if XV[g]:
                    t1 = end[("pv", g - 1)] if g + 1 < HKV else end[("qk", g)] + 8
                    tasks.append([qb_task(g), REP, start[("qk", g)] - 20, start[("qk", g)] - 4, 0, None])
                    tasks.append([kq_task(g), XV[g] // XT * 16, start[("qk", g)], t1, 0, None])
            for g in range(HKV):
                st = ("qk", g + 1) if g + 1 < HKV else ("pv", g - 1)
                tasks.append([sm_task(g), NT // 2 // SMG, end[st] - SMA, end[st] - SMB, 0, None])

            def pinned(lhs, key=None):
                tau = clock[0]
                bits = None
                for tk in tasks:
                    gen, n, t0, t1, done = tk[:5]
                    if tau < t0 or done > n:
                        continue
                    want = n + 1 if tau >= t1 else (n * (tau - t0 + 1)) // (t1 - t0)
                    while tk[4] < want:
                        pin = next(gen, None)
                        tk[4] += 1
                        if pin is not None:
                            tk[5] = pin
                    if tau % PG == PG - 1 and tk[5] is not None:
                        pin = tk[5][(tau // PG) % len(tk[5])]
                        tk[5] = None
                        pb = pltpu.bitcast(pin, u32)
                        bits = pb if bits is None else bits | pb
                clock[0] += 1
                if bits is not None:
                    return pltpu.bitcast(pltpu.bitcast(lhs, u32) | (bits & zmask), f32).astype(bf16)
                if key is None:
                    return lhs.astype(bf16)
                if key not in qpk:
                    qpk[key] = lhs.astype(bf16)
                return qpk[key]

            for kind, g in stages:
                if kind == "qk":
                    for t in range(NT - XV[g]):
                        d = mm(pinned(qs[g][t % 2], (g, t % 2)), k_u[g, t * 64:(t + 1) * 64, :])
                        res.append(d)
                        ss[g][t // 2] = _acc(ss[g][t // 2], d)
                else:
                    acc = [None] * 4
                    for t in range(NT):
                        lhs = pinned(ps[g][t // 2], ("p", g, t // 2))
                        if g < HKV - 1 or t < VPK:
                            d = mm(lhs, v_u[g, t * 64:(t + 1) * 64, :])
                        else:
                            d = jnp.dot(lhs, v1buf[g, t * 128:(t + 1) * 128, :], preferred_element_type=f32)
                        res.append(d)
                        acc[t % 4] = _acc(acc[t % 4], d)
                    o = ((acc[0] + acc[2]) + pltpu.roll(acc[1] + acc[3], 1, 0)) / ls[g]
                    if g < HKV - 1:
                        ob16 = _rnd(o)[1]
                        for r in range(REP):
                            ob_sc[g][r] = colb(ob16[ROWS[r]:ROWS[r] + 1, :])
            clock[0] += O6L
            for tk in tasks:
                for _ in tk[0]:
                    pass
            x1 = (xf + rowsum(jnp.concatenate(yacc, axis=1))) + wo_last(o)
            x1, _ = ffn_fast(x1, m, zmask)
            o_ref[1:2, :] = x1[0:1, :].astype(o_ref.dtype)

        pl.run_scoped(batch1, pltpu.VMEM((HKV, SK // 2, DH), u32), pltpu.VMEM((HKV, SK // 2, DH), u32))

    pl.run_scoped(whole, pltpu.SemaphoreType.DMA((NSEM,)))


@jax.jit
def pallas_interleave_layers__gqa_block_cached__dense_activation_silu__decode_kernel(A_x, A_k_cache, A_v_cache, A_wq, A_wo, B_x, B_w1, B_w2):
    x2 = A_x.reshape(B, D)
    any_spec = pl.BlockSpec(memory_space=pl.ANY)
    out = pl.pallas_call(
        _kernel,
        out_shape=jax.ShapeDtypeStruct((B, D), bf16),
        in_specs=[any_spec] * 7,
        out_specs=pl.BlockSpec(memory_space=pltpu.VMEM),
        scratch_shapes=[
            pltpu.VMEM((B, D), bf16),
            pltpu.VMEM((HKV, SK, DH), bf16),
            pltpu.VMEM((HKV, SK, DH), bf16),
            pltpu.VMEM((D, HQ * DH), bf16),
            pltpu.VMEM((HQ * DH, D), bf16),
            pltpu.VMEM((D, F), bf16),
            pltpu.VMEM((F, D), bf16),
            pltpu.VMEM((HQ, D // 2, 128), u32),
            pltpu.VMEM((ND, HQ * DH // 2, 128), u32),
            pltpu.VMEM((NJ, D // 2, 128), u32),
            pltpu.VMEM((ND, F // 2, 128), u32),
            pltpu.VMEM((HQ, D, 128), f32),
            pltpu.VMEM((HQ, DH, D), f32),
            pltpu.VMEM((HV * 128, D), f32),
            pltpu.VMEM((HV * 128, D), f32),
            pltpu.VMEM((HKV, 8, DH), f32),
            pltpu.VMEM((8, F), f32),
            pltpu.VMEM((B, HKV, 8, DH), bf16),
            pltpu.VMEM((HKV, 8, SK), bf16),
            pltpu.VMEM((HKV, 8, DH), f32),
            pltpu.VMEM((8, D), f32),
            pltpu.VMEM((D, 128), f32),
            pltpu.SMEM((1,), jnp.int32),
            pltpu.VMEM((HKV, XVMAX * 128, 128), f32),
        ] + [pltpu.VMEM((REP, DH, 128), f32)] * (2 * HKV - 1),
        compiler_params=pltpu.CompilerParams(vmem_limit_bytes=116 * 1024 * 1024),
    )(x2, A_k_cache, A_v_cache, A_wq, A_wo, B_w1, B_w2)
    return out.reshape(B, 1, D)
```
